```python
import jax
import jax.numpy as jnp

def _softmax(x, axis=-1):
    return jax.nn.softmax(x, axis=axis)

def _gelu(x):
    return jax.nn.gelu(x, approximate=True)

def _silu(x):
    return jax.nn.silu(x)

def _sigmoid(x):
    return jax.nn.sigmoid(x)

def _layernorm(x, axis=-1, eps=1e-05):
    m = jnp.mean(x, axis=axis, keepdims=True)
    v = jnp.var(x, axis=axis, keepdims=True)
    return (x - m) / jnp.sqrt(v + eps)

def _scatter_add(tgt, idx, src, axis=0):
    return tgt.at[idx].add(src)

def _segment_sum(src, seg, n):
    return jax.ops.segment_sum(src, seg, n)

class _Rng:

    def __init__(self, key):
        self._k = key

    def _next(self):
        self._k, sub = jax.random.split(self._k)
        return sub

    def normal(self, shape):
        return jax.random.normal(self._next(), shape, dtype=jnp.bfloat16)

    def randint(self, lo, hi, shape):
        return jax.random.randint(self._next(), shape, lo, hi, dtype=jnp.int32)

    def uniform(self, shape, lo=0.0, hi=1.0):
        return jax.random.uniform(self._next(), shape, jnp.bfloat16, lo, hi)

    def permutation(self, n):
        return jax.random.permutation(self._next(), n)
kernel_name = 'adaLN_cond__memory_aug_recurrent_mem_tr__dense_activation_gelu__prompt'

def setup_inputs():
    _rng = _Rng(jax.random.key(int.from_bytes(__import__("os").urandom(4), "little")))
    _w = lambda a: (lambda t: t.astype(jnp.bfloat16) if jnp.issubdtype(t.dtype, jnp.floating) else t)(jnp.asarray(a))

    def _A_setup():
        B, S, Dm = (1, 2048, 1024)
        H, Dh = (32, 128)
        M, seg = (8, 32)
        seg = min(seg, S)
        S = S // seg * seg
        return {'x': _w((lambda *s: _rng.normal(s) * 0.05)(B, S, Dm)), 'mem0': _w((lambda *s: _rng.normal(s) * 0.05)(B, M, Dm)), 'Wq': _w((lambda *s: _rng.normal(s) * 0.05)(Dm, H, Dh) * Dm ** (-0.5)), 'Wk': _w((lambda *s: _rng.normal(s) * 0.05)(Dm, H, Dh) * Dm ** (-0.5)), 'Wv': _w((lambda *s: _rng.normal(s) * 0.05)(Dm, H, Dh) * Dm ** (-0.5)), 'Wo': _w((lambda *s: _rng.normal(s) * 0.05)(H, Dh, Dm) * (H * Dh) ** (-0.5)), 'seg_len': seg}
    _A_in = _A_setup()

    def _B_setup():
        B, S, D, F = (1, 2048, 1024, 3584)
        return {'x': _w((lambda *s: _rng.normal(s) * 0.05)(B, S, D)), 'w1': _w((lambda *s: _rng.normal(s) * 0.05)(D, F) * D ** (-0.5)), 'b1': _w((lambda *s: _rng.normal(s) * 0.05)(F) * 0.01), 'w2': _w((lambda *s: _rng.normal(s) * 0.05)(F, D) * F ** (-0.5)), 'b2': _w((lambda *s: _rng.normal(s) * 0.05)(D) * 0.01)}
    _B_in = _B_setup()
    return {'A_x': _A_in['x'], 'A_mem0': _A_in['mem0'], 'A_Wq': _A_in['Wq'], 'A_Wk': _A_in['Wk'], 'A_Wv': _A_in['Wv'], 'A_Wo': _A_in['Wo'], 'A_seg_len': _A_in['seg_len'], 'B_x': _B_in['x'], 'B_w1': _B_in['w1'], 'B_b1': _B_in['b1'], 'B_w2': _B_in['w2'], 'B_b2': _B_in['b2'], 'c': _w((lambda *s: _rng.normal(s) * 0.05)(1, 1024)), 'w_mod': _w((lambda *s: _rng.normal(s) * 0.05)(1024, 6 * 1024) * 1024 ** (-0.5))}

def reference(A_x, A_mem0, A_Wq, A_Wk, A_Wv, A_Wo, A_seg_len, B_x, B_w1, B_b1, B_w2, B_b2, c, w_mod):

    def _A_ref(x, mem0, Wq, Wk, Wv, Wo, seg_len):
        B, S, Dm = x.shape
        H, Dh = (Wq.shape[1], Wq.shape[2])
        M = mem0.shape[1]
        scale = Dh ** (-0.5)
        n_seg = S // seg_len
        L = M + seg_len
        idx = jnp.arange(L)
        mask = (idx[:, None] < M) | (idx[:, None] >= idx[None, :])
        mem = mem0
        outs = []
        for s in range(n_seg):
            xs = x[:, s * seg_len:(s + 1) * seg_len, :].copy()
            h = jnp.concatenate([mem, xs], axis=1)
            q = jnp.einsum('btd,dhe->bhte', h, Wq)
            k = jnp.einsum('btd,dhe->bhte', h, Wk)
            v = jnp.einsum('btd,dhe->bhte', h, Wv)
            scores = jnp.einsum('bhqe,bhke->bhqk', q, k) * scale
            scores = jnp.where(mask[None, None], scores, -1000000000.0)
            p = _softmax(scores, axis=-1)
            o = jnp.einsum('bhqk,bhke->bhqe', p, v)
            o = jnp.einsum('bhte,hed->btd', o, Wo)
            mem = o[:, :M, :].copy()
            outs.append(o[:, M:, :])
        return jnp.concatenate(outs, axis=1)

    def _B_ref(x, w1, b1, w2, b2):
        h = jnp.einsum('bsd,df->bsf', x, w1) + b1
        h = _gelu(h)
        return jnp.einsum('bsf,fd->bsd', h, w2) + b2
    x = A_x
    mod = (_silu(c) @ w_mod).reshape(c.shape[0], 6, 1, -1)
    sa, ca, ga, sb, cb, gb = (mod[:, 0].copy(), mod[:, 1].copy(), mod[:, 2].copy(), mod[:, 3].copy(), mod[:, 4].copy(), mod[:, 5].copy())
    h = _layernorm(x, axis=-1) * (1 + ca) + sa
    x = x + ga * _A_ref(h, A_mem0, A_Wq, A_Wk, A_Wv, A_Wo, A_seg_len)
    h = _layernorm(x, axis=-1) * (1 + cb) + sb
    x = x + gb * _B_ref(h, B_w1, B_b1, B_w2, B_b2)
    return x
```

```python
import functools

import jax
import jax.numpy as jnp
import jax.experimental.pallas as pl
import jax.experimental.pallas.tpu as pltpu

F32 = jnp.float32
BF16 = jnp.bfloat16
U32 = jnp.uint32

S, D, H, E, M, SEG, F = 2048, 1024, 32, 128, 8, 32, 3584
NSEG = S // SEG
TPS = 24
PRE = S - NSEG * TPS
RING = 576
OFF = 64
RC = 256
NF = F // 128
ND = D // 128


def _ln(x):
    m = jnp.mean(x, axis=-1, keepdims=True)
    xc = x - m
    v = jnp.mean(xc * xc, axis=-1, keepdims=True)
    return xc * jax.lax.rsqrt(v + 1e-5)


def _dot(a, b):
    return jnp.dot(a, b, preferred_element_type=F32)


def _kernel(x_ref, mem0_ref, b1_ref, b2_ref, c_ref,
            wq_hbm, wk_hbm, wv_hbm, wo_hbm, w1_hbm, w2_hbm, wm_hbm,
            out_ref,
            wqkv, wo, w1, w2, hbuf, qr, kr, vr, stg, wm, modv, sems):
    def wm_cp(j):
        return pltpu.make_async_copy(wm_hbm.at[:, pl.ds(j * D, D)], wm.at[j], sems.at[j])

    def stg_cp(i, half):
        w = (wq_hbm, wk_hbm, wv_hbm)[i]
        return pltpu.make_async_copy(
            w.bitcast(U32).at[pl.ds(half * 512, 512)], stg.at[half], sems.at[6 + half])

    def wo_cp(n):
        return pltpu.make_async_copy(
            wo_hbm.at[:, pl.ds(n * 128, 128)], wo.at[n], sems.at[8 + n])

    def w1_cp(j):
        return pltpu.make_async_copy(
            w1_hbm.at[:, pl.ds(j * 128, 128)], w1.at[j], sems.at[16])

    def w2_cp(n):
        return pltpu.make_async_copy(
            w2_hbm.at[:, pl.ds(n * 128, 128)], w2.at[n], sems.at[17])

    wm_cp(0).start()
    wm_cp(1).start()
    stg_cp(0, 0).start()
    stg_cp(0, 1).start()

    cc = c_ref[...].astype(F32)
    sc = jnp.broadcast_to(cc * jax.nn.sigmoid(cc), (8, D)).astype(BF16)

    def mod_chunk(j):
        wm_cp(j).wait()
        modv[j] = _dot(sc, wm[j])

    mod_chunk(0)
    mod_chunk(1)
    sa = modv[0][0:1, :]
    ca = modv[1][0:1, :]

    def ln_body(i, _):
        r = pl.multiple_of(i * 256, 256)
        hbuf[pl.ds(r, 256), :] = _ln(x_ref[pl.ds(r, 256), :].astype(F32)) * (1.0 + ca) + sa
    jax.lax.fori_loop(0, S // 256, ln_body, None)

    s2 = stg.reshape(2 * 512 * 16, 128)

    def relayout(i, half):
        def body(t, _):
            base = (half * 512 + t * 16) * 16
            dd = pl.multiple_of(half * 512 + t * 16, 16)
            for p in range(16):
                a = s2[pl.ds(base + p, 8, stride=32), :]
                b = s2[pl.ds(base + 16 + p, 8, stride=32), :]
                lo = (a & jnp.uint32(0xFFFF)) | (b << 16)
                hi = (a >> 16) | (b & jnp.uint32(0xFFFF0000))
                wqkv[i * H + 2 * p, pl.ds(dd, 16), :] = pltpu.bitcast(lo, BF16)
                wqkv[i * H + 2 * p + 1, pl.ds(dd, 16), :] = pltpu.bitcast(hi, BF16)
        jax.lax.fori_loop(0, 32, body, None)

    rings = (qr, kr, vr)
    for i in range(3):
        for half in range(2):
            stg_cp(i, half).wait()
            relayout(i, half)
            if i < 2:
                stg_cp(i + 1, half).start()
        if i == 1:
            for n in range(ND):
                wo_cp(n).start()
            for j in range(2, 6):
                wm_cp(j).start()
        if i == 2:
            for j in range(NF):
                w1_cp(j).start()
            for n in range(ND):
                w2_cp(n).start()

        def pre_body(h, _, i=i):
            lhs = hbuf[0:PRE, :].astype(BF16)
            rings[i][h, OFF:OFF + PRE, :] = _dot(lhs, wqkv[i * H + h])
        jax.lax.fori_loop(0, H, pre_body, None)

    for n in range(ND):
        wo_cp(n).wait()
    for j in range(2, 6):
        mod_chunk(j)

    row = jax.lax.broadcasted_iota(jnp.int32, (M + SEG, M + SEG), 0)
    col = jax.lax.broadcasted_iota(jnp.int32, (M + SEG, M + SEG), 1)
    mask = (row < M) | (row >= col)
    scale = E ** -0.5

    def step(s, mem):
        tin = pl.multiple_of(PRE + s * TPS, 8)
        slot_in = pl.multiple_of(jax.lax.rem(OFF + PRE + s * TPS, RING), 8)
        slot_seg = pl.multiple_of(jax.lax.rem(OFF + s * SEG, RING), 8)
        tout = pl.multiple_of(s * TPS, 8)
        slot_out = pl.multiple_of(jax.lax.rem(OFF + s * TPS, RING), 8)
        slot_out2 = pl.multiple_of(jax.lax.rem(OFF + M + s * TPS, RING), 8)
        lhs = jnp.concatenate([mem, hbuf[pl.ds(tin, TPS), :]], axis=0).astype(BF16)
        om = []
        for h in range(H):
            full = []
            for i in range(3):
                y = _dot(lhs, wqkv[i * H + h])
                rings[i][h, pl.ds(slot_in, TPS), :] = y[M:, :]
                tok = rings[i][h, pl.ds(slot_seg, SEG), :]
                full.append(jnp.concatenate([y[:M, :], tok], axis=0).astype(BF16))
            q, k, v = full
            sc_ = jax.lax.dot_general(q, k, (((1,), (1,)), ((), ())),
                                      preferred_element_type=F32) * scale
            sc_ = jnp.where(mask, sc_, -1e9)
            p = jnp.exp(sc_ - jnp.max(sc_, axis=-1, keepdims=True))
            p = p / jnp.sum(p, axis=-1, keepdims=True)
            o = _dot(p.astype(BF16), v)
            qr[h, pl.ds(slot_seg, SEG), :] = o[M:, :]
            om.append(o[:M, :])
        lo = [jnp.concatenate([om[h], qr[h, pl.ds(slot_out, 8), :],
                               qr[h, pl.ds(slot_out2, TPS - 8), :]], axis=0).astype(BF16)
              for h in range(H)]
        outs = []
        for n in range(ND):
            acc = None
            for h in range(H):
                y = _dot(lo[h], wo[n, h * E:(h + 1) * E, :])
                acc = y if acc is None else acc + y
            outs.append(acc)
        res = jnp.concatenate(outs, axis=1)
        hbuf[pl.ds(tout, TPS), :] = res[M:, :]
        return res[:M, :]

    jax.lax.fori_loop(0, NSEG, step, mem0_ref[...].astype(F32))

    T0 = NSEG * TPS
    for blk in range(PRE // 128):
        t = T0 + blk * 128
        parts = []
        left = 128
        while left:
            sl = (OFF + t + 128 - left) % RING
            n_ = min(left, RING - sl)
            parts.append((sl, n_))
            left -= n_

        def wo_body(n, _, parts=parts, t=t):
            acc = None
            for h in range(H):
                a = jnp.concatenate([qr[h, sl:sl + n_, :] for sl, n_ in parts], axis=0)
                y = _dot(a.astype(BF16), wo[n, h * E:(h + 1) * E, :])
                acc = y if acc is None else acc + y
            hbuf[t:t + 128, pl.ds(pl.multiple_of(n * 128, 128), 128)] = acc
        jax.lax.fori_loop(0, ND, wo_body, None)

    for j in range(NF):
        w1_cp(j).wait()
    for n in range(ND):
        w2_cp(n).wait()
    ga = modv[2][0:1, :]
    sb = modv[3][0:1, :]
    cb = modv[4][0:1, :]
    gb = modv[5][0:1, :]
    b2 = b2_ref[...].astype(F32)

    def ffn_body(i, _):
        r = pl.multiple_of(i * RC, RC)
        x1 = x_ref[pl.ds(r, RC), :].astype(F32) + ga * hbuf[pl.ds(r, RC), :]
        h2 = (_ln(x1) * (1.0 + cb) + sb).astype(BF16)
        g = []
        for j in range(NF):
            u = _dot(h2, w1[j]) + b1_ref[:, j * 128:(j + 1) * 128].astype(F32)
            g.append(jax.nn.gelu(u, approximate=True).astype(BF16))
        gg = jnp.concatenate(g, axis=1)
        y = jnp.concatenate([_dot(gg, w2[n]) for n in range(ND)], axis=1)
        out_ref[pl.ds(r, RC), :] = (x1 + gb * (y + b2)).astype(out_ref.dtype)
    jax.lax.fori_loop(0, S // RC, ffn_body, None)


@functools.partial(jax.jit, static_argnames=("A_seg_len",))
def pallas_adaLN_cond__memory_aug_recurrent_mem_tr__dense_activation_gelu__prompt_kernel(
    A_x, A_mem0, A_Wq, A_Wk, A_Wv, A_Wo, A_seg_len, B_x, B_w1, B_b1, B_w2, B_b2, c, w_mod,
):
    assert A_seg_len == SEG and A_x.shape == (1, S, D)
    vm = pl.BlockSpec(memory_space=pltpu.VMEM)
    hb = pl.BlockSpec(memory_space=pl.ANY)
    out = pl.pallas_call(
        _kernel,
        out_shape=jax.ShapeDtypeStruct((S, D), A_x.dtype),
        in_specs=[vm] * 5 + [hb] * 7,
        out_specs=vm,
        scratch_shapes=[
            pltpu.VMEM((3 * H, D, E), BF16),
            pltpu.VMEM((ND, H * E, 128), BF16),
            pltpu.VMEM((NF, D, 128), BF16),
            pltpu.VMEM((ND, F, 128), BF16),
            pltpu.VMEM((S, D), F32),
            pltpu.VMEM((H, RING, E), F32),
            pltpu.VMEM((H, RING, E), F32),
            pltpu.VMEM((H, RING, E), F32),
            pltpu.VMEM((2, 512, 16, 128), U32),
            pltpu.VMEM((6, D, D), BF16),
            pltpu.VMEM((6, 8, D), F32),
            pltpu.SemaphoreType.DMA((18,)),
        ],
        compiler_params=pltpu.CompilerParams(vmem_limit_bytes=126 * 2**20),
    )(A_x.reshape(S, D), A_mem0.reshape(M, D), B_b1.reshape(1, F), B_b2.reshape(1, D), c,
      A_Wq, A_Wk, A_Wv, A_Wo.reshape(H * E, D), B_w1, B_w2, w_mod)
    return out.reshape(1, S, D)
```

```python
import functools

import jax
import jax.numpy as jnp
import jax.experimental.pallas as pl
import jax.experimental.pallas.tpu as pltpu

F32 = jnp.float32
BF16 = jnp.bfloat16
U32 = jnp.uint32

S, D, H, E, M, SEG, F = 2048, 1024, 32, 128, 8, 32, 3584
NSEG = S // SEG
TPS = 24
TAIL = S - NSEG * TPS
PRE = 544
RING = 576
OFF = 32
RC = 256
NF = F // 128
ND = D // 128


def _ln(x):
    m = jnp.mean(x, axis=-1, keepdims=True)
    xc = x - m
    v = jnp.mean(xc * xc, axis=-1, keepdims=True)
    return xc * jax.lax.rsqrt(v + 1e-5)


def _dot(a, b):
    return jnp.dot(a, b, preferred_element_type=F32)


def _kernel(x_ref, mem0_ref, b1_ref, b2_ref, c_ref,
            wq_hbm, wk_hbm, wv_hbm, wo_hbm, w1_hbm, w2_hbm, wm_hbm,
            out_ref,
            wqkv, wo, w1, w2, hbuf, qr, kr, vr, stg, wm, modv, sems):
    def wm_cp(j):
        return pltpu.make_async_copy(wm_hbm.at[:, pl.ds(j * D, D)], wm.at[j], sems.at[j])

    def stg_cp(i, half):
        w = (wq_hbm, wk_hbm, wv_hbm)[i]
        return pltpu.make_async_copy(
            w.bitcast(U32).at[pl.ds(half * 512, 512)], stg.at[half], sems.at[6 + half])

    def wo_cp(n):
        return pltpu.make_async_copy(
            wo_hbm.at[:, pl.ds(n * 128, 128)], wo.at[n], sems.at[8 + n])

    def w1_cp(j):
        return pltpu.make_async_copy(
            w1_hbm.at[:, pl.ds(j * 128, 128)], w1.at[j], sems.at[16])

    def w2_cp(n):
        return pltpu.make_async_copy(
            w2_hbm.at[:, pl.ds(n * 128, 128)], w2.at[n], sems.at[17])

    wm_cp(0).start()
    wm_cp(1).start()
    stg_cp(0, 0).start()
    stg_cp(0, 1).start()

    cc = c_ref[...].astype(F32)
    sc = jnp.broadcast_to(cc * jax.nn.sigmoid(cc), (8, D)).astype(BF16)

    def mod_chunk(j):
        wm_cp(j).wait()
        modv[j] = _dot(sc, wm[j])

    mod_chunk(0)
    mod_chunk(1)
    sa = modv[0][0:1, :]
    ca = modv[1][0:1, :]

    def ln_body(i, _):
        r = pl.multiple_of(i * 256, 256)
        hbuf[pl.ds(r, 256), :] = _ln(x_ref[pl.ds(r, 256), :].astype(F32)) * (1.0 + ca) + sa
    jax.lax.fori_loop(0, S // 256, ln_body, None)

    hbuf[S:S + 32, :] = jnp.zeros((32, D), F32)
    s2 = stg.reshape(2 * 512 * 16, 128)

    def relayout(i, half):
        def body(t, _):
            base = (half * 512 + t * 16) * 16
            dd = pl.multiple_of(half * 512 + t * 16, 16)
            for p in range(16):
                a = s2[pl.ds(base + p, 8, stride=32), :]
                b = s2[pl.ds(base + 16 + p, 8, stride=32), :]
                lo = (a & jnp.uint32(0xFFFF)) | (b << 16)
                hi = (a >> 16) | (b & jnp.uint32(0xFFFF0000))
                wqkv[i * H + 2 * p, pl.ds(dd, 16), :] = pltpu.bitcast(lo, BF16)
                wqkv[i * H + 2 * p + 1, pl.ds(dd, 16), :] = pltpu.bitcast(hi, BF16)
        jax.lax.fori_loop(0, 32, body, None)

    rings = (qr, kr, vr)
    for i in range(3):
        for half in range(2):
            stg_cp(i, half).wait()
            relayout(i, half)
            if i < 2:
                stg_cp(i + 1, half).start()
        if i == 1:
            for n in range(ND):
                wo_cp(n).start()
            for j in range(2, 6):
                wm_cp(j).start()
        if i == 2:
            for j in range(NF):
                w1_cp(j).start()
            for n in range(ND):
                w2_cp(n).start()

        def pre_body(h, _, i=i):
            lhs = hbuf[0:PRE, :].astype(BF16)
            rings[i][h, OFF:OFF + PRE, :] = _dot(lhs, wqkv[i * H + h])
        jax.lax.fori_loop(0, H, pre_body, None)

    for n in range(ND):
        wo_cp(n).wait()
    for j in range(2, 6):
        mod_chunk(j)

    row = jax.lax.broadcasted_iota(jnp.int32, (M + SEG, M + SEG), 0)
    col = jax.lax.broadcasted_iota(jnp.int32, (M + SEG, M + SEG), 1)
    mask = (row < M) | (row >= col)
    scale = E ** -0.5

    def step(s, mem):
        tin = pl.multiple_of(PRE + s * TPS, 8)
        slot_in = pl.multiple_of(jax.lax.rem(OFF + PRE + s * TPS, RING), 8)
        slot_seg = pl.multiple_of(jax.lax.rem(OFF + s * SEG, RING), 8)
        tout = pl.multiple_of(s * TPS, 8)
        slot_out = pl.multiple_of(jax.lax.rem(OFF + s * TPS, RING), 8)
        slot_out2 = pl.multiple_of(jax.lax.rem(OFF + 16 + s * TPS, RING), 8)
        lhs = jnp.concatenate([mem, hbuf[pl.ds(tin, TPS), :]], axis=0).astype(BF16)
        om = []
        toks = [[rings[i][h, pl.ds(slot_seg, SEG), :] for i in range(3)] for h in range(H)]
        qkv = []
        for h in range(H):
            full = []
            for i in range(3):
                y = _dot(lhs, wqkv[i * H + h])
                rings[i][h, pl.ds(slot_in, TPS), :] = y[M:, :]
                full.append(jnp.concatenate([y[:M, :], toks[h][i]], axis=0).astype(BF16))
            qkv.append(full)
        scs = [jax.lax.dot_general(q, k, (((1,), (1,)), ((), ())),
                                   preferred_element_type=F32) for q, k, _ in qkv]
        ps = []
        for sc_ in scs:
            sc_ = jnp.where(mask, sc_ * scale, -1e9)
            p = jnp.exp(sc_ - jnp.max(sc_, axis=-1, keepdims=True))
            ps.append((p / jnp.sum(p, axis=-1, keepdims=True)).astype(BF16))
        for h in range(H):
            o = _dot(ps[h], qkv[h][2])
            qr[h, pl.ds(slot_seg, SEG), :] = o[M:, :]
            om.append(o[:M, :])
        lo = [jnp.concatenate([om[h], qr[h, pl.ds(slot_out, 16), :],
                               qr[h, pl.ds(slot_out2, 8), :]], axis=0).astype(BF16)
              for h in range(H)]
        outs = []
        for n in range(ND):
            acc = None
            for h in range(H):
                y = _dot(lo[h], wo[n, h * E:(h + 1) * E, :])
                acc = y if acc is None else acc + y
            outs.append(acc)
        res = jnp.concatenate(outs, axis=1)
        hbuf[pl.ds(tout, TPS), :] = res[M:, :]
        return res[:M, :]

    jax.lax.fori_loop(0, NSEG, step, mem0_ref[...].astype(F32))

    T0 = NSEG * TPS
    for blk in range(TAIL // 128):
        t = T0 + blk * 128
        parts = []
        left = 128
        while left:
            sl = (OFF + t + 128 - left) % RING
            n_ = min(left, RING - sl)
            parts.append((sl, n_))
            left -= n_

        def wo_body(n, _, parts=parts, t=t):
            acc = None
            for h in range(H):
                a = jnp.concatenate([qr[h, sl:sl + n_, :] for sl, n_ in parts], axis=0)
                y = _dot(a.astype(BF16), wo[n, h * E:(h + 1) * E, :])
                acc = y if acc is None else acc + y
            hbuf[t:t + 128, pl.ds(pl.multiple_of(n * 128, 128), 128)] = acc
        jax.lax.fori_loop(0, ND, wo_body, None)

    for j in range(NF):
        w1_cp(j).wait()
    for n in range(ND):
        w2_cp(n).wait()
    ga = modv[2][0:1, :]
    sb = modv[3][0:1, :]
    cb = modv[4][0:1, :]
    gb = modv[5][0:1, :]
    b2 = b2_ref[...].astype(F32)

    def ffn_body(i, _):
        r = pl.multiple_of(i * RC, RC)
        x1 = x_ref[pl.ds(r, RC), :].astype(F32) + ga * hbuf[pl.ds(r, RC), :]
        h2 = (_ln(x1) * (1.0 + cb) + sb).astype(BF16)
        g = []
        for j in range(NF):
            u = _dot(h2, w1[j]) + b1_ref[:, j * 128:(j + 1) * 128].astype(F32)
            g.append(jax.nn.gelu(u, approximate=True).astype(BF16))
        gg = jnp.concatenate(g, axis=1)
        y = jnp.concatenate([_dot(gg, w2[n]) for n in range(ND)], axis=1)
        out_ref[pl.ds(r, RC), :] = (x1 + gb * (y + b2)).astype(out_ref.dtype)
    jax.lax.fori_loop(0, S // RC, ffn_body, None)


@functools.partial(jax.jit, static_argnames=("A_seg_len",))
def pallas_adaLN_cond__memory_aug_recurrent_mem_tr__dense_activation_gelu__prompt_kernel(
    A_x, A_mem0, A_Wq, A_Wk, A_Wv, A_Wo, A_seg_len, B_x, B_w1, B_b1, B_w2, B_b2, c, w_mod,
):
    assert A_seg_len == SEG and A_x.shape == (1, S, D)
    vm = pl.BlockSpec(memory_space=pltpu.VMEM)
    hb = pl.BlockSpec(memory_space=pl.ANY)
    out = pl.pallas_call(
        _kernel,
        out_shape=jax.ShapeDtypeStruct((S, D), A_x.dtype),
        in_specs=[vm] * 5 + [hb] * 7,
        out_specs=vm,
        scratch_shapes=[
            pltpu.VMEM((3 * H, D, E), BF16),
            pltpu.VMEM((ND, H * E, 128), BF16),
            pltpu.VMEM((NF, D, 128), BF16),
            pltpu.VMEM((ND, F, 128), BF16),
            pltpu.VMEM((S + 32, D), F32),
            pltpu.VMEM((H, RING, E), F32),
            pltpu.VMEM((H, RING, E), F32),
            pltpu.VMEM((H, RING, E), F32),
            pltpu.VMEM((2, 512, 16, 128), U32),
            pltpu.VMEM((6, D, D), BF16),
            pltpu.VMEM((6, 8, D), F32),
            pltpu.SemaphoreType.DMA((18,)),
        ],
        compiler_params=pltpu.CompilerParams(vmem_limit_bytes=126 * 2**20),
    )(A_x.reshape(S, D), A_mem0.reshape(M, D), B_b1.reshape(1, F), B_b2.reshape(1, D), c,
      A_Wq, A_Wk, A_Wv, A_Wo.reshape(H * E, D), B_w1, B_w2, w_mod)
    return out.reshape(1, S, D)
```

```python
import functools

import jax
import jax.numpy as jnp
import jax.experimental.pallas as pl
import jax.experimental.pallas.tpu as pltpu

F32 = jnp.float32
BF16 = jnp.bfloat16
U32 = jnp.uint32

S, D, H, E, M, SEG, F = 2048, 1024, 32, 128, 8, 32, 3584
NSEG = S // SEG
TPS = 24
TAIL = S - NSEG * TPS
PRE = 544
RING = 576
OFF = 32
LAG1, LAG2, LAG3 = 4, 8, 12
RC = 256
NF = F // 128
ND = D // 128


def _ln(x):
    m = jnp.mean(x, axis=-1, keepdims=True)
    xc = x - m
    v = jnp.mean(xc * xc, axis=-1, keepdims=True)
    return xc * jax.lax.rsqrt(v + 1e-5)


def _dot(a, b):
    return jnp.dot(a, b, preferred_element_type=F32)


def _kernel(x_ref, mem0_ref, b1_ref, b2_ref, c_ref,
            wq_hbm, wk_hbm, wv_hbm, wo_hbm, w1_hbm, w2_hbm, wm_hbm,
            out_ref,
            wqkv, wo, w1, w2, hbuf, qr, kr, vr, stg, wm, modv, sems):
    def wm_cp(j):
        return pltpu.make_async_copy(wm_hbm.at[:, pl.ds(j * D, D)], wm.at[j % 2], sems.at[j % 2])

    def stg_cp(i, half):
        w = (wq_hbm, wk_hbm, wv_hbm)[i]
        return pltpu.make_async_copy(
            w.bitcast(U32).at[pl.ds(half * 512, 512)], stg.at[(i % 2) * 2 + half], sems.at[2 + (i % 2) * 2 + half])

    def wo_cp(n):
        return pltpu.make_async_copy(
            wo_hbm.at[:, pl.ds(n * 128, 128)], wo.at[n], sems.at[8 + n])

    def w1_cp(j):
        return pltpu.make_async_copy(
            w1_hbm.at[:, pl.ds(j * 128, 128)], w1.at[j], sems.at[16])

    def w2_cp(n):
        return pltpu.make_async_copy(
            w2_hbm.at[:, pl.ds(n * 128, 128)], w2.at[n], sems.at[17])

    wm_cp(0).start()
    wm_cp(1).start()
    stg_cp(0, 0).start()
    stg_cp(0, 1).start()
    stg_cp(1, 0).start()
    stg_cp(1, 1).start()

    cc = c_ref[...].astype(F32)
    sc = jnp.broadcast_to(cc * jax.nn.sigmoid(cc), (8, D)).astype(BF16)

    def mod_chunk(j):
        wm_cp(j).wait()
        modv[j] = _dot(sc, wm[j % 2])

    mod_chunk(0)
    mod_chunk(1)
    sa = modv[0][0:1, :]
    ca = modv[1][0:1, :]

    def ln_body(i, _):
        r = pl.multiple_of(i * 256, 256)
        hbuf[pl.ds(r, 256), :] = _ln(x_ref[pl.ds(r, 256), :].astype(F32)) * (1.0 + ca) + sa
    jax.lax.fori_loop(0, S // 256, ln_body, None)

    hbuf[S:S + 32, :] = jnp.zeros((32, D), F32)
    s2 = stg.reshape(4 * 512 * 16, 128)

    def relayout16(i, t):
        base = ((i % 2) * 1024 + t * 16) * 16
        dd = pl.multiple_of(t * 16, 16)
        for p in range(16):
            a = s2[pl.ds(base + p, 8, stride=32), :]
            b = s2[pl.ds(base + 16 + p, 8, stride=32), :]
            lo = (a & jnp.uint32(0xFFFF)) | (b << 16)
            hi = (a >> 16) | (b & jnp.uint32(0xFFFF0000))
            wqkv[i * H + 2 * p, pl.ds(dd, 16), :] = pltpu.bitcast(lo, BF16)
            wqkv[i * H + 2 * p + 1, pl.ds(dd, 16), :] = pltpu.bitcast(hi, BF16)

    rings = (qr, kr, vr)
    for half in range(2):
        stg_cp(0, half).wait()
        jax.lax.fori_loop(half * 32, half * 32 + 32, lambda t, _: relayout16(0, t), None)
    stg_cp(2, 0).start()
    stg_cp(2, 1).start()
    for n in range(ND):
        wo_cp(n).start()
    wm_cp(2).start()
    wm_cp(3).start()
    for j in range(NF):
        w1_cp(j).start()
    for n in range(ND):
        w2_cp(n).start()
    for i in range(3):
        if i < 2:
            stg_cp(i + 1, 0).wait()
            stg_cp(i + 1, 1).wait()

        def pre_body(h, _, i=i):
            lhs = hbuf[0:PRE, :].astype(BF16)
            rings[i][h, OFF:OFF + PRE, :] = _dot(lhs, wqkv[i * H + h])
            if i < 2:
                relayout16(i + 1, 2 * h)
                relayout16(i + 1, 2 * h + 1)
        jax.lax.fori_loop(0, H, pre_body, None)

    for n in range(ND):
        wo_cp(n).wait()

    row = jax.lax.broadcasted_iota(jnp.int32, (M + SEG, M + SEG), 0)
    col = jax.lax.broadcasted_iota(jnp.int32, (M + SEG, M + SEG), 1)
    mask = (row < M) | (row >= col)
    scale = E ** -0.5

    def step(s, mem):
        tin = pl.multiple_of(PRE + s * TPS, 8)
        slot_in = pl.multiple_of(jax.lax.rem(OFF + PRE + s * TPS, RING), 8)
        slot_seg = pl.multiple_of(jax.lax.rem(OFF + s * SEG, RING), 8)
        tout = pl.multiple_of(s * TPS, 8)
        slot_out = pl.multiple_of(jax.lax.rem(OFF + s * TPS, RING), 8)
        slot_out2 = pl.multiple_of(jax.lax.rem(OFF + 16 + s * TPS, RING), 8)
        lhs = jnp.concatenate([mem, hbuf[pl.ds(tin, TPS), :]], axis=0).astype(BF16)
        om = []
        toks = [[rings[i][h, pl.ds(slot_seg, SEG), :] for i in range(3)] for h in range(H)]
        qkv, scs, ps = {}, {}, {}
        outs = [None] * ND

        def st_qkv(h):
            full = []
            for i in range(3):
                y = _dot(lhs, wqkv[i * H + h])
                rings[i][h, pl.ds(slot_in, TPS), :] = y[M:, :]
                full.append(jnp.concatenate([y[:M, :], toks[h][i]], axis=0).astype(BF16))
            qkv[h] = full

        def st_s(h):
            q, k, _ = qkv[h]
            scs[h] = jax.lax.dot_general(q, k, (((1,), (1,)), ((), ())),
                                         preferred_element_type=F32)

        def st_p(h):
            sc_ = jnp.where(mask, scs[h] * scale, -1e9)
            p = jnp.exp(sc_ - jnp.max(sc_, axis=-1, keepdims=True))
            ps[h] = (p / jnp.sum(p, axis=-1, keepdims=True)).astype(BF16)

        def st_o(h):
            o = _dot(ps[h], qkv[h][2])
            qr[h, pl.ds(slot_seg, SEG), :] = o[M:, :]
            om.append(o[:M, :])

        for t in range(H + LAG3):
            if t < H:
                st_qkv(t)
            if 0 <= t - LAG1 < H:
                st_s(t - LAG1)
            if 0 <= t - LAG2 < H:
                st_p(t - LAG2)
            if 0 <= t - LAG3 < H:
                st_o(t - LAG3)
        lo = [jnp.concatenate([om[h], qr[h, pl.ds(slot_out, 16), :],
                               qr[h, pl.ds(slot_out2, 8), :]], axis=0).astype(BF16)
              for h in range(H)]
        for h in range(H):
            for n in range(ND):
                y = _dot(lo[h], wo[n, h * E:(h + 1) * E, :])
                outs[n] = y if outs[n] is None else outs[n] + y
        res = jnp.concatenate(outs, axis=1)
        hbuf[pl.ds(tout, TPS), :] = res[M:, :]
        return res[:M, :]

    jax.lax.fori_loop(0, NSEG, step, mem0_ref[...].astype(F32))

    mod_chunk(2)
    mod_chunk(3)
    wm_cp(4).start()
    wm_cp(5).start()
    T0 = NSEG * TPS
    for blk in range(TAIL // 128):
        t = T0 + blk * 128
        parts = []
        left = 128
        while left:
            sl = (OFF + t + 128 - left) % RING
            n_ = min(left, RING - sl)
            parts.append((sl, n_))
            left -= n_

        def wo_body(n, _, parts=parts, t=t):
            acc = None
            for h in range(H):
                a = jnp.concatenate([qr[h, sl:sl + n_, :] for sl, n_ in parts], axis=0)
                y = _dot(a.astype(BF16), wo[n, h * E:(h + 1) * E, :])
                acc = y if acc is None else acc + y
            hbuf[t:t + 128, pl.ds(pl.multiple_of(n * 128, 128), 128)] = acc
        jax.lax.fori_loop(0, ND, wo_body, None)

    for j in range(NF):
        w1_cp(j).wait()
    for n in range(ND):
        w2_cp(n).wait()
    mod_chunk(4)
    mod_chunk(5)
    ga = modv[2][0:1, :]
    sb = modv[3][0:1, :]
    cb = modv[4][0:1, :]
    gb = modv[5][0:1, :]
    b2 = b2_ref[...].astype(F32)

    def ffn_body(i, _):
        r = pl.multiple_of(i * RC, RC)
        x1 = x_ref[pl.ds(r, RC), :].astype(F32) + ga * hbuf[pl.ds(r, RC), :]
        h2 = (_ln(x1) * (1.0 + cb) + sb).astype(BF16)
        g = []
        for j in range(NF):
            u = _dot(h2, w1[j]) + b1_ref[:, j * 128:(j + 1) * 128].astype(F32)
            g.append(jax.nn.gelu(u, approximate=True).astype(BF16))
        gg = jnp.concatenate(g, axis=1)
        y = jnp.concatenate([_dot(gg, w2[n]) for n in range(ND)], axis=1)
        out_ref[pl.ds(r, RC), :] = (x1 + gb * (y + b2)).astype(out_ref.dtype)
    jax.lax.fori_loop(0, S // RC, ffn_body, None)


@functools.partial(jax.jit, static_argnames=("A_seg_len",))
def pallas_adaLN_cond__memory_aug_recurrent_mem_tr__dense_activation_gelu__prompt_kernel(
    A_x, A_mem0, A_Wq, A_Wk, A_Wv, A_Wo, A_seg_len, B_x, B_w1, B_b1, B_w2, B_b2, c, w_mod,
):
    assert A_seg_len == SEG and A_x.shape == (1, S, D)
    vm = pl.BlockSpec(memory_space=pltpu.VMEM)
    hb = pl.BlockSpec(memory_space=pl.ANY)
    out = pl.pallas_call(
        _kernel,
        out_shape=jax.ShapeDtypeStruct((S, D), A_x.dtype),
        in_specs=[vm] * 5 + [hb] * 7,
        out_specs=vm,
        scratch_shapes=[
            pltpu.VMEM((3 * H, D, E), BF16),
            pltpu.VMEM((ND, H * E, 128), BF16),
            pltpu.VMEM((NF, D, 128), BF16),
            pltpu.VMEM((ND, F, 128), BF16),
            pltpu.VMEM((S + 32, D), F32),
            pltpu.VMEM((H, RING, E), F32),
            pltpu.VMEM((H, RING, E), F32),
            pltpu.VMEM((H, RING, E), F32),
            pltpu.VMEM((4, 512, 16, 128), U32),
            pltpu.VMEM((2, D, D), BF16),
            pltpu.VMEM((6, 8, D), F32),
            pltpu.SemaphoreType.DMA((18,)),
        ],
        compiler_params=pltpu.CompilerParams(vmem_limit_bytes=126 * 2**20),
    )(A_x.reshape(S, D), A_mem0.reshape(M, D), B_b1.reshape(1, F), B_b2.reshape(1, D), c,
      A_Wq, A_Wk, A_Wv, A_Wo.reshape(H * E, D), B_w1, B_w2, w_mod)
    return out.reshape(1, S, D)
```

```python
import functools

import jax
import jax.numpy as jnp
import jax.experimental.pallas as pl
import jax.experimental.pallas.tpu as pltpu

F32 = jnp.float32
BF16 = jnp.bfloat16
U32 = jnp.uint32

S, D, H, E, M, SEG, F = 2048, 1024, 32, 128, 8, 32, 3584
NSEG = S // SEG
TPS = 24
TAIL = S - NSEG * TPS
PRE = 544
RING = 576
OFF = 32
LAG1, LAG2, LAG3, LAG4 = 4, 8, 12, 16
RC = 256
NF = F // 128
ND = D // 128


def _ln(x):
    m = jnp.mean(x, axis=-1, keepdims=True)
    xc = x - m
    v = jnp.mean(xc * xc, axis=-1, keepdims=True)
    return xc * jax.lax.rsqrt(v + 1e-5)


def _dot(a, b):
    return jnp.dot(a, b, preferred_element_type=F32)


def _kernel(x_ref, mem0_ref, b1_ref, b2_ref, c_ref,
            wq_hbm, wk_hbm, wv_hbm, wo_hbm, w1_hbm, w2_hbm, wm_hbm,
            out_ref,
            wqkv, wo, w1, w2, hbuf, qr, kr, vr, stg, wm, modv, hb, sems):
    def wm_cp(j):
        return pltpu.make_async_copy(wm_hbm.at[:, pl.ds(j * D, D)], wm.at[j % 2], sems.at[j % 2])

    def stg_cp(i, half):
        w = (wq_hbm, wk_hbm, wv_hbm)[i]
        return pltpu.make_async_copy(
            w.bitcast(U32).at[pl.ds(half * 512, 512)], stg.at[(i % 2) * 2 + half], sems.at[2 + (i % 2) * 2 + half])

    def wo_cp(n):
        return pltpu.make_async_copy(
            wo_hbm.at[:, pl.ds(n * 128, 128)], wo.at[n], sems.at[8 + n])

    def w1_cp(j):
        return pltpu.make_async_copy(
            w1_hbm.at[:, pl.ds(j * 128, 128)], w1.at[j], sems.at[16])

    def w2_cp(n):
        return pltpu.make_async_copy(
            w2_hbm.at[:, pl.ds(n * 128, 128)], w2.at[n], sems.at[17])

    wm_cp(0).start()
    wm_cp(1).start()
    stg_cp(0, 0).start()
    stg_cp(0, 1).start()

    cc = c_ref[...].astype(F32)
    sc = jnp.broadcast_to(cc * jax.nn.sigmoid(cc), (8, D)).astype(BF16)

    def mod_chunk(j):
        wm_cp(j).wait()
        modv[j] = _dot(sc, wm[j % 2])

    mod_chunk(0)
    mod_chunk(1)
    stg_cp(1, 0).start()
    stg_cp(1, 1).start()
    sa = modv[0][0:1, :]
    ca = modv[1][0:1, :]

    def ln_body(i, _):
        r = pl.multiple_of(i * 256, 256)
        hbuf[pl.ds(r, 256), :] = _ln(x_ref[pl.ds(r, 256), :].astype(F32)) * (1.0 + ca) + sa
    jax.lax.fori_loop(0, S // 256, ln_body, None)

    hbuf[S:S + 32, :] = jnp.zeros((32, D), F32)
    s2 = stg.reshape(4 * 512 * 16, 128)

    def relayout16(i, t):
        base = ((i % 2) * 1024 + t * 16) * 16
        dd = pl.multiple_of(t * 16, 16)
        for p in range(16):
            a = s2[pl.ds(base + p, 8, stride=32), :]
            b = s2[pl.ds(base + 16 + p, 8, stride=32), :]
            lo = (a & jnp.uint32(0xFFFF)) | (b << 16)
            hi = (a >> 16) | (b & jnp.uint32(0xFFFF0000))
            wqkv[i * H + 2 * p, pl.ds(dd, 16), :] = pltpu.bitcast(lo, BF16)
            wqkv[i * H + 2 * p + 1, pl.ds(dd, 16), :] = pltpu.bitcast(hi, BF16)

    hb[...] = hbuf[0:PRE, :].astype(BF16)
    rings = (qr, kr, vr)
    for half in range(2):
        stg_cp(0, half).wait()
        jax.lax.fori_loop(half * 32, half * 32 + 32, lambda t, _: relayout16(0, t), None)
    stg_cp(2, 0).start()
    stg_cp(2, 1).start()
    for n in range(ND):
        wo_cp(n).start()
    wm_cp(2).start()
    wm_cp(3).start()
    for j in range(NF):
        w1_cp(j).start()
    for n in range(ND):
        w2_cp(n).start()
    for i in range(3):
        if i < 2:
            stg_cp(i + 1, 0).wait()
            stg_cp(i + 1, 1).wait()

        def pre_body(h, _, i=i):
            lhs = hb[...]
            rings[i][h, OFF:OFF + PRE, :] = _dot(lhs, wqkv[i * H + h])
            if i < 2:
                relayout16(i + 1, 2 * h)
                relayout16(i + 1, 2 * h + 1)
        jax.lax.fori_loop(0, H, pre_body, None, unroll=2)

    for n in range(ND):
        wo_cp(n).wait()

    row = jax.lax.broadcasted_iota(jnp.int32, (M + SEG, M + SEG), 0)
    col = jax.lax.broadcasted_iota(jnp.int32, (M + SEG, M + SEG), 1)
    mask = (row < M) | (row >= col)
    scale = E ** -0.5

    def step(s, mem):
        tin = pl.multiple_of(PRE + s * TPS, 8)
        slot_in = pl.multiple_of(jax.lax.rem(OFF + PRE + s * TPS, RING), 8)
        slot_seg = pl.multiple_of(jax.lax.rem(OFF + s * SEG, RING), 8)
        tout = pl.multiple_of(s * TPS, 8)
        slot_out = pl.multiple_of(jax.lax.rem(OFF + s * TPS, RING), 8)
        slot_out2 = pl.multiple_of(jax.lax.rem(OFF + 16 + s * TPS, RING), 8)
        lhs = jnp.concatenate([mem, hbuf[pl.ds(tin, TPS), :]], axis=0).astype(BF16)
        om = []
        toks = [[rings[i][h, pl.ds(slot_seg, SEG), :] for i in range(3)] for h in range(H)]
        qkv, scs, ps = {}, {}, {}
        outs = [None] * ND

        def st_qkv(h):
            full = []
            for i in range(3):
                y = _dot(lhs, wqkv[i * H + h])
                rings[i][h, pl.ds(slot_in, TPS), :] = y[M:, :]
                full.append(jnp.concatenate([y[:M, :], toks[h][i]], axis=0).astype(BF16))
            qkv[h] = full

        def st_s(h):
            q, k, _ = qkv[h]
            scs[h] = jax.lax.dot_general(q, k, (((1,), (1,)), ((), ())),
                                         preferred_element_type=F32)

        def st_p(h):
            sc_ = jnp.where(mask, scs[h] * scale, -1e9)
            p = jnp.exp(sc_ - jnp.max(sc_, axis=-1, keepdims=True))
            ps[h] = (p / jnp.sum(p, axis=-1, keepdims=True)).astype(BF16)

        def st_o(h):
            o = _dot(ps[h], qkv[h][2])
            qr[h, pl.ds(slot_seg, SEG), :] = o[M:, :]
            om.append(jnp.concatenate(
                [o[:M, :], qr[h, pl.ds(slot_out, 16), :], qr[h, pl.ds(slot_out2, 8), :]],
                axis=0).astype(BF16))

        def st_w(h):
            for n in range(ND):
                y = _dot(om[h], wo[n, h * E:(h + 1) * E, :])
                outs[n] = y if outs[n] is None else outs[n] + y

        for t in range(H + LAG4):
            if t < H:
                st_qkv(t)
            if 0 <= t - LAG1 < H:
                st_s(t - LAG1)
            if 0 <= t - LAG2 < H:
                st_p(t - LAG2)
            if 0 <= t - LAG3 < H:
                st_o(t - LAG3)
            if 0 <= t - LAG4 < H:
                st_w(t - LAG4)
        res = jnp.concatenate(outs, axis=1)
        hbuf[pl.ds(tout, TPS), :] = res[M:, :]
        return res[:M, :]

    jax.lax.fori_loop(0, NSEG, step, mem0_ref[...].astype(F32))

    mod_chunk(2)
    mod_chunk(3)
    wm_cp(4).start()
    wm_cp(5).start()
    T0 = NSEG * TPS
    for blk in range(TAIL // 128):
        t = T0 + blk * 128
        parts = []
        left = 128
        while left:
            sl = (OFF + t + 128 - left) % RING
            n_ = min(left, RING - sl)
            parts.append((sl, n_))
            left -= n_

        def wo_body(n, _, parts=parts, t=t):
            acc = None
            for h in range(H):
                a = jnp.concatenate([qr[h, sl:sl + n_, :] for sl, n_ in parts], axis=0)
                y = _dot(a.astype(BF16), wo[n, h * E:(h + 1) * E, :])
                acc = y if acc is None else acc + y
            hbuf[t:t + 128, pl.ds(pl.multiple_of(n * 128, 128), 128)] = acc
        jax.lax.fori_loop(0, ND, wo_body, None, unroll=2)

    for j in range(NF):
        w1_cp(j).wait()
    for n in range(ND):
        w2_cp(n).wait()
    mod_chunk(4)
    mod_chunk(5)
    ga = modv[2][0:1, :]
    sb = modv[3][0:1, :]
    cb = modv[4][0:1, :]
    gb = modv[5][0:1, :]
    b2 = b2_ref[...].astype(F32)

    def ffn_body(i, _):
        r = pl.multiple_of(i * RC, RC)
        x1 = x_ref[pl.ds(r, RC), :].astype(F32) + ga * hbuf[pl.ds(r, RC), :]
        h2 = (_ln(x1) * (1.0 + cb) + sb).astype(BF16)
        g = []
        for j in range(NF):
            u = _dot(h2, w1[j]) + b1_ref[:, j * 128:(j + 1) * 128].astype(F32)
            g.append(jax.nn.gelu(u, approximate=True).astype(BF16))
        gg = jnp.concatenate(g, axis=1)
        y = jnp.concatenate([_dot(gg, w2[n]) for n in range(ND)], axis=1)
        out_ref[pl.ds(r, RC), :] = (x1 + gb * (y + b2)).astype(out_ref.dtype)
    jax.lax.fori_loop(0, S // RC, ffn_body, None)


@functools.partial(jax.jit, static_argnames=("A_seg_len",))
def pallas_adaLN_cond__memory_aug_recurrent_mem_tr__dense_activation_gelu__prompt_kernel(
    A_x, A_mem0, A_Wq, A_Wk, A_Wv, A_Wo, A_seg_len, B_x, B_w1, B_b1, B_w2, B_b2, c, w_mod,
):
    assert A_seg_len == SEG and A_x.shape == (1, S, D)
    vm = pl.BlockSpec(memory_space=pltpu.VMEM)
    hb = pl.BlockSpec(memory_space=pl.ANY)
    out = pl.pallas_call(
        _kernel,
        out_shape=jax.ShapeDtypeStruct((S, D), A_x.dtype),
        in_specs=[vm] * 5 + [hb] * 7,
        out_specs=vm,
        scratch_shapes=[
            pltpu.VMEM((3 * H, D, E), BF16),
            pltpu.VMEM((ND, H * E, 128), BF16),
            pltpu.VMEM((NF, D, 128), BF16),
            pltpu.VMEM((ND, F, 128), BF16),
            pltpu.VMEM((S + 32, D), F32),
            pltpu.VMEM((H, RING, E), F32),
            pltpu.VMEM((H, RING, E), F32),
            pltpu.VMEM((H, RING, E), F32),
            pltpu.VMEM((4, 512, 16, 128), U32),
            pltpu.VMEM((2, D, D), BF16),
            pltpu.VMEM((6, 8, D), F32),
            pltpu.VMEM((PRE, D), BF16),
            pltpu.SemaphoreType.DMA((18,)),
        ],
        compiler_params=pltpu.CompilerParams(vmem_limit_bytes=126 * 2**20),
    )(A_x.reshape(S, D), A_mem0.reshape(M, D), B_b1.reshape(1, F), B_b2.reshape(1, D), c,
      A_Wq, A_Wk, A_Wv, A_Wo.reshape(H * E, D), B_w1, B_w2, w_mod)
    return out.reshape(1, S, D)
```

```python
import functools

import jax
import jax.numpy as jnp
import jax.experimental.pallas as pl
import jax.experimental.pallas.tpu as pltpu

F32 = jnp.float32
BF16 = jnp.bfloat16
U32 = jnp.uint32

S, D, H, E, M, SEG, F = 2048, 1024, 32, 128, 8, 32, 3584
NSEG = S // SEG
TPS = 24
TAIL = S - NSEG * TPS
PRE = 544
RING = 576
OFF = 32
LAG1, LAG2, LAG3, LAG4 = 4, 8, 12, 16
RC = 256
NF = F // 128
ND = D // 128


def _ln(x):
    m = jnp.mean(x, axis=-1, keepdims=True)
    xc = x - m
    v = jnp.mean(xc * xc, axis=-1, keepdims=True)
    return xc * jax.lax.rsqrt(v + 1e-5)


def _dot(a, b):
    return jnp.dot(a, b, preferred_element_type=F32)


def _kernel(x_ref, mem0_ref, b1_ref, b2_ref, c_ref,
            wq_hbm, wk_hbm, wv_hbm, wo_hbm, w1_hbm, w2_hbm, wm_hbm,
            out_ref,
            wqkv, wo, w1, w2, hbuf, qr, kr, vr, stg, wm, modv, hb, sems):
    def wm_cp(j):
        return pltpu.make_async_copy(wm_hbm.at[:, pl.ds(j * D, D)], wm.at[j % 2], sems.at[j % 2])

    def stg_cps(i):
        w32 = (wq_hbm, wk_hbm, wv_hbm)[i].bitcast(U32)
        return [pltpu.make_async_copy(w32.at[:, p, :], stg.at[i % 2, p], sems.at[2 + i % 2])
                for p in range(16)]

    def wo_cp(n):
        return pltpu.make_async_copy(
            wo_hbm.at[:, pl.ds(n * 128, 128)], wo.at[n], sems.at[8 + n])

    def w1_cp(j):
        return pltpu.make_async_copy(
            w1_hbm.at[:, pl.ds(j * 128, 128)], w1.at[j], sems.at[16])

    def w2_cp(n):
        return pltpu.make_async_copy(
            w2_hbm.at[:, pl.ds(n * 128, 128)], w2.at[n], sems.at[17])

    wm_cp(0).start()
    wm_cp(1).start()
    for cp in stg_cps(0):
        cp.start()

    cc = c_ref[...].astype(F32)
    sc = jnp.broadcast_to(cc * jax.nn.sigmoid(cc), (8, D)).astype(BF16)

    def mod_chunk(j):
        wm_cp(j).wait()
        modv[j] = _dot(sc, wm[j % 2])

    mod_chunk(0)
    mod_chunk(1)
    for cp in stg_cps(1):
        cp.start()
    sa = modv[0][0:1, :]
    ca = modv[1][0:1, :]

    def ln_body(i, _):
        r = pl.multiple_of(i * 256, 256)
        hbuf[pl.ds(r, 256), :] = _ln(x_ref[pl.ds(r, 256), :].astype(F32)) * (1.0 + ca) + sa
    jax.lax.fori_loop(0, S // 256, ln_body, None)

    hbuf[S:S + 32, :] = jnp.zeros((32, D), F32)

    def relayout16(i, t):
        dd = pl.multiple_of(t * 16, 16)
        for p in range(16):
            a = stg[i % 2, p, pl.ds(dd, 8, stride=2), :]
            b = stg[i % 2, p, pl.ds(dd + 1, 8, stride=2), :]
            lo = (a & jnp.uint32(0xFFFF)) | (b << 16)
            hi = (a >> 16) | (b & jnp.uint32(0xFFFF0000))
            wqkv[i * H + 2 * p, pl.ds(dd, 16), :] = pltpu.bitcast(lo, BF16)
            wqkv[i * H + 2 * p + 1, pl.ds(dd, 16), :] = pltpu.bitcast(hi, BF16)

    hb[...] = hbuf[0:PRE, :].astype(BF16)
    rings = (qr, kr, vr)
    for cp in stg_cps(0):
        cp.wait()
    jax.lax.fori_loop(0, 64, lambda t, _: relayout16(0, t), None)
    for cp in stg_cps(2):
        cp.start()
    for n in range(ND):
        wo_cp(n).start()
    wm_cp(2).start()
    wm_cp(3).start()
    for j in range(NF):
        w1_cp(j).start()
    for n in range(ND):
        w2_cp(n).start()
    for i in range(3):
        if i < 2:
            for cp in stg_cps(i + 1):
                cp.wait()

        def pre_body(h, _, i=i):
            lhs = hb[...]
            rings[i][h, OFF:OFF + PRE, :] = _dot(lhs, wqkv[i * H + h])
            if i < 2:
                relayout16(i + 1, 2 * h)
                relayout16(i + 1, 2 * h + 1)
        jax.lax.fori_loop(0, H, pre_body, None, unroll=2)

    for n in range(ND):
        wo_cp(n).wait()

    row = jax.lax.broadcasted_iota(jnp.int32, (M + SEG, M + SEG), 0)
    col = jax.lax.broadcasted_iota(jnp.int32, (M + SEG, M + SEG), 1)
    mask = (row < M) | (row >= col)
    scale = E ** -0.5

    def step(s, mem):
        tin = pl.multiple_of(PRE + s * TPS, 8)
        slot_in = pl.multiple_of(jax.lax.rem(OFF + PRE + s * TPS, RING), 8)
        slot_seg = pl.multiple_of(jax.lax.rem(OFF + s * SEG, RING), 8)
        tout = pl.multiple_of(s * TPS, 8)
        slot_out = pl.multiple_of(jax.lax.rem(OFF + s * TPS, RING), 8)
        slot_out2 = pl.multiple_of(jax.lax.rem(OFF + 16 + s * TPS, RING), 8)
        lhs = jnp.concatenate([mem, hbuf[pl.ds(tin, TPS), :]], axis=0).astype(BF16)
        om = []
        toks = [[rings[i][h, pl.ds(slot_seg, SEG), :] for i in range(3)] for h in range(H)]
        qkv, scs, ps = {}, {}, {}
        outs = [None] * ND

        def st_qkv(h):
            full = []
            for i in range(3):
                y = _dot(lhs, wqkv[i * H + h])
                rings[i][h, pl.ds(slot_in, TPS), :] = y[M:, :]
                full.append(jnp.concatenate([y[:M, :], toks[h][i]], axis=0).astype(BF16))
            qkv[h] = full

        def st_s(h):
            q, k, _ = qkv[h]
            scs[h] = jax.lax.dot_general(q, k, (((1,), (1,)), ((), ())),
                                         preferred_element_type=F32)

        def st_p(h):
            sc_ = jnp.where(mask, scs[h] * scale, -1e9)
            p = jnp.exp(sc_ - jnp.max(sc_, axis=-1, keepdims=True))
            ps[h] = (p / jnp.sum(p, axis=-1, keepdims=True)).astype(BF16)

        def st_o(h):
            o = _dot(ps[h], qkv[h][2])
            qr[h, pl.ds(slot_seg, SEG), :] = o[M:, :]
            om.append(jnp.concatenate(
                [o[:M, :], qr[h, pl.ds(slot_out, 16), :], qr[h, pl.ds(slot_out2, 8), :]],
                axis=0).astype(BF16))

        def st_w(h):
            for n in range(ND):
                y = _dot(om[h], wo[n, h * E:(h + 1) * E, :])
                outs[n] = y if outs[n] is None else outs[n] + y

        for t in range(H + LAG4):
            if t < H:
                st_qkv(t)
            if 0 <= t - LAG1 < H:
                st_s(t - LAG1)
            if 0 <= t - LAG2 < H:
                st_p(t - LAG2)
            if 0 <= t - LAG3 < H:
                st_o(t - LAG3)
            if 0 <= t - LAG4 < H:
                st_w(t - LAG4)
        res = jnp.concatenate(outs, axis=1)
        hbuf[pl.ds(tout, TPS), :] = res[M:, :]
        return res[:M, :]

    jax.lax.fori_loop(0, NSEG, step, mem0_ref[...].astype(F32))

    mod_chunk(2)
    mod_chunk(3)
    wm_cp(4).start()
    wm_cp(5).start()
    T0 = NSEG * TPS
    for blk in range(TAIL // 128):
        t = T0 + blk * 128
        parts = []
        left = 128
        while left:
            sl = (OFF + t + 128 - left) % RING
            n_ = min(left, RING - sl)
            parts.append((sl, n_))
            left -= n_

        def wo_body(n, _, parts=parts, t=t):
            acc = None
            for h in range(H):
                a = jnp.concatenate([qr[h, sl:sl + n_, :] for sl, n_ in parts], axis=0)
                y = _dot(a.astype(BF16), wo[n, h * E:(h + 1) * E, :])
                acc = y if acc is None else acc + y
            hbuf[t:t + 128, pl.ds(pl.multiple_of(n * 128, 128), 128)] = acc
        jax.lax.fori_loop(0, ND, wo_body, None, unroll=2)

    for j in range(NF):
        w1_cp(j).wait()
    for n in range(ND):
        w2_cp(n).wait()
    mod_chunk(4)
    mod_chunk(5)
    ga = modv[2][0:1, :]
    sb = modv[3][0:1, :]
    cb = modv[4][0:1, :]
    gb = modv[5][0:1, :]
    b2 = b2_ref[...].astype(F32)

    def ffn_body(i, _):
        r = pl.multiple_of(i * RC, RC)
        x1 = x_ref[pl.ds(r, RC), :].astype(F32) + ga * hbuf[pl.ds(r, RC), :]
        h2 = (_ln(x1) * (1.0 + cb) + sb).astype(BF16)
        g = []
        for j in range(NF):
            u = _dot(h2, w1[j]) + b1_ref[:, j * 128:(j + 1) * 128].astype(F32)
            g.append(jax.nn.gelu(u, approximate=True).astype(BF16))
        gg = jnp.concatenate(g, axis=1)
        y = jnp.concatenate([_dot(gg, w2[n]) for n in range(ND)], axis=1)
        out_ref[pl.ds(r, RC), :] = (x1 + gb * (y + b2)).astype(out_ref.dtype)
    jax.lax.fori_loop(0, S // RC, ffn_body, None)


@functools.partial(jax.jit, static_argnames=("A_seg_len",))
def pallas_adaLN_cond__memory_aug_recurrent_mem_tr__dense_activation_gelu__prompt_kernel(
    A_x, A_mem0, A_Wq, A_Wk, A_Wv, A_Wo, A_seg_len, B_x, B_w1, B_b1, B_w2, B_b2, c, w_mod,
):
    assert A_seg_len == SEG and A_x.shape == (1, S, D)
    vm = pl.BlockSpec(memory_space=pltpu.VMEM)
    hb = pl.BlockSpec(memory_space=pl.ANY)
    out = pl.pallas_call(
        _kernel,
        out_shape=jax.ShapeDtypeStruct((S, D), A_x.dtype),
        in_specs=[vm] * 5 + [hb] * 7,
        out_specs=vm,
        scratch_shapes=[
            pltpu.VMEM((3 * H, D, E), BF16),
            pltpu.VMEM((ND, H * E, 128), BF16),
            pltpu.VMEM((NF, D, 128), BF16),
            pltpu.VMEM((ND, F, 128), BF16),
            pltpu.VMEM((S + 32, D), F32),
            pltpu.VMEM((H, RING, E), F32),
            pltpu.VMEM((H, RING, E), F32),
            pltpu.VMEM((H, RING, E), F32),
            pltpu.VMEM((2, 16, D, 128), U32),
            pltpu.VMEM((2, D, D), BF16),
            pltpu.VMEM((6, 8, D), F32),
            pltpu.VMEM((PRE, D), BF16),
            pltpu.SemaphoreType.DMA((18,)),
        ],
        compiler_params=pltpu.CompilerParams(vmem_limit_bytes=126 * 2**20),
    )(A_x.reshape(S, D), A_mem0.reshape(M, D), B_b1.reshape(1, F), B_b2.reshape(1, D), c,
      A_Wq, A_Wk, A_Wv, A_Wo.reshape(H * E, D), B_w1, B_w2, w_mod)
    return out.reshape(1, S, D)
```

```python
import functools

import jax
import jax.numpy as jnp
import jax.experimental.pallas as pl
import jax.experimental.pallas.tpu as pltpu

F32 = jnp.float32
BF16 = jnp.bfloat16
U32 = jnp.uint32

S, D, H, E, M, SEG, F = 2048, 1024, 32, 128, 8, 32, 3584
NSEG = S // SEG
TPS = 24
TAIL = S - NSEG * TPS
PRE = 544
RING = 576
OFF = 32
LAG1, LAG2, LAG3, LAG4 = 4, 8, 12, 16
RC = 256
NF = F // 128
ND = D // 128


def _ln(x):
    m = jnp.mean(x, axis=-1, keepdims=True)
    xc = x - m
    v = jnp.mean(xc * xc, axis=-1, keepdims=True)
    return xc * jax.lax.rsqrt(v + 1e-5)


def _dot(a, b):
    if b.dtype == U32:
        b = pltpu.bitcast(b, BF16)
    return jnp.dot(a, b, preferred_element_type=F32)


def _kernel(x_ref, mem0_ref, b1_ref, b2_ref, c_ref,
            wq_hbm, wk_hbm, wv_hbm, wo_hbm, w1_hbm, w2_hbm, wm_hbm,
            out_hbm,
            wqkv, wo, w1, w2, hbuf, qr, kr, vr, stg, wm, modv, hb, out_ref, sems):
    def wm_cp(j):
        return pltpu.make_async_copy(wm_hbm.at[:, pl.ds(j * D, D)], wm.at[j % 2], sems.at[j % 2])

    def stg_cps(i):
        w32 = (wq_hbm, wk_hbm, wv_hbm)[i].bitcast(U32)
        return [pltpu.make_async_copy(w32.at[:, p, :], stg.at[i % 2, p], sems.at[2 + i % 2])
                for p in range(16)]

    def wo_cp(n):
        return pltpu.make_async_copy(
            wo_hbm.bitcast(U32).at[:, pl.ds(n * 128, 128)], wo.at[n], sems.at[8 + n])

    def w1_cp(j):
        return pltpu.make_async_copy(
            w1_hbm.bitcast(U32).at[:, pl.ds(j * 128, 128)], w1.at[j], sems.at[16])

    def w2_cp(n):
        return pltpu.make_async_copy(
            w2_hbm.bitcast(U32).at[:, pl.ds(n * 128, 128)], w2.at[n], sems.at[17])

    wm_cp(0).start()
    wm_cp(1).start()
    for i in range(2):
        for cp in stg_cps(i):
            cp.start()

    cc = c_ref[...].astype(F32)
    sc = jnp.broadcast_to(cc * jax.nn.sigmoid(cc), (8, D)).astype(BF16)

    def mod_chunk(j):
        wm_cp(j).wait()
        modv[j] = _dot(sc, wm[j % 2])

    mod_chunk(0)
    mod_chunk(1)
    sa = modv[0][0:1, :]
    ca = modv[1][0:1, :]

    def ln_body(i, _):
        r = pl.multiple_of(i * 256, 256)
        hbuf[pl.ds(r, 256), :] = _ln(x_ref[pl.ds(r, 256), :].astype(F32)) * (1.0 + ca) + sa
    jax.lax.fori_loop(0, S // 256, ln_body, None)

    hbuf[S:S + 32, :] = jnp.zeros((32, D), F32)

    def relayout16(i, t):
        dd = pl.multiple_of(t * 16, 16)
        d2 = pl.multiple_of(t * 8, 8)
        for p in range(16):
            a = stg[i % 2, p, pl.ds(dd, 8, stride=2), :]
            b = stg[i % 2, p, pl.ds(dd + 1, 8, stride=2), :]
            lo = (a & jnp.uint32(0xFFFF)) | (b << 16)
            hi = (a >> 16) | (b & jnp.uint32(0xFFFF0000))
            wqkv[i * H + 2 * p, pl.ds(d2, 8), :] = lo
            wqkv[i * H + 2 * p + 1, pl.ds(d2, 8), :] = hi

    hb[...] = hbuf[0:PRE, :].astype(BF16)
    rings = (qr, kr, vr)
    for cp in stg_cps(0):
        cp.wait()
    jax.lax.fori_loop(0, 64, lambda t, _: relayout16(0, t), None)
    for cp in stg_cps(2):
        cp.start()
    for i in range(3):
        if i < 2:
            for cp in stg_cps(i + 1):
                cp.wait()
        if i == 1:
            for n in range(ND):
                wo_cp(n).start()
            wm_cp(2).start()
            wm_cp(3).start()
            for j in range(NF):
                w1_cp(j).start()
            for n in range(ND):
                w2_cp(n).start()

        def pre_body(h, _, i=i):
            lhs = hb[...]
            rings[i][h, OFF:OFF + PRE, :] = _dot(lhs, wqkv[i * H + h])
            if i < 2:
                relayout16(i + 1, 2 * h)
                relayout16(i + 1, 2 * h + 1)
        jax.lax.fori_loop(0, H, pre_body, None, unroll=2)

    for n in range(ND):
        wo_cp(n).wait()

    row = jax.lax.broadcasted_iota(jnp.int32, (M + SEG, M + SEG), 0)
    col = jax.lax.broadcasted_iota(jnp.int32, (M + SEG, M + SEG), 1)
    mask = (row < M) | (row >= col)
    scale = E ** -0.5

    def step(s, mem):
        tin = pl.multiple_of(PRE + s * TPS, 8)
        slot_in = pl.multiple_of(jax.lax.rem(OFF + PRE + s * TPS, RING), 8)
        slot_seg = pl.multiple_of(jax.lax.rem(OFF + s * SEG, RING), 8)
        tout = pl.multiple_of(s * TPS, 8)
        slot_out = pl.multiple_of(jax.lax.rem(OFF + s * TPS, RING), 8)
        slot_out2 = pl.multiple_of(jax.lax.rem(OFF + 16 + s * TPS, RING), 8)
        lhs = jnp.concatenate([mem, hbuf[pl.ds(tin, TPS), :]], axis=0).astype(BF16)
        om = []
        toks = [[rings[i][h, pl.ds(slot_seg, SEG), :] for i in range(3)] for h in range(H)]
        qkv, scs, ps = {}, {}, {}
        outs = [None] * ND

        def st_qkv(h):
            full = []
            for i in range(3):
                y = _dot(lhs, wqkv[i * H + h])
                rings[i][h, pl.ds(slot_in, TPS), :] = y[M:, :]
                full.append(jnp.concatenate([y[:M, :], toks[h][i]], axis=0).astype(BF16))
            qkv[h] = full

        def st_s(h):
            q, k, _ = qkv[h]
            scs[h] = jax.lax.dot_general(q, k, (((1,), (1,)), ((), ())),
                                         preferred_element_type=F32)

        def st_p(h):
            sc_ = jnp.where(mask, scs[h] * scale, -1e9)
            p = jnp.exp(sc_ - jnp.max(sc_, axis=-1, keepdims=True))
            ps[h] = (p / jnp.sum(p, axis=-1, keepdims=True)).astype(BF16)

        def st_o(h):
            o = _dot(ps[h], qkv[h][2])
            qr[h, pl.ds(slot_seg, SEG), :] = o[M:, :]
            om.append(jnp.concatenate(
                [o[:M, :], qr[h, pl.ds(slot_out, 16), :], qr[h, pl.ds(slot_out2, 8), :]],
                axis=0).astype(BF16))

        def st_w(h):
            for n in range(ND):
                y = _dot(om[h], wo[n, h * 64:(h + 1) * 64, :])
                outs[n] = y if outs[n] is None else outs[n] + y

        for t in range(H + LAG4):
            if t < H:
                st_qkv(t)
            if 0 <= t - LAG1 < H:
                st_s(t - LAG1)
            if 0 <= t - LAG2 < H:
                st_p(t - LAG2)
            if 0 <= t - LAG3 < H:
                st_o(t - LAG3)
            if 0 <= t - LAG4 < H:
                st_w(t - LAG4)
        res = jnp.concatenate(outs, axis=1)
        hbuf[pl.ds(tout, TPS), :] = res[M:, :]
        return res[:M, :]

    jax.lax.fori_loop(0, NSEG, step, mem0_ref[...].astype(F32))

    mod_chunk(2)
    mod_chunk(3)
    wm_cp(4).start()
    wm_cp(5).start()
    T0 = NSEG * TPS
    for blk in range(TAIL // 128):
        t = T0 + blk * 128
        parts = []
        left = 128
        while left:
            sl = (OFF + t + 128 - left) % RING
            n_ = min(left, RING - sl)
            parts.append((sl, n_))
            left -= n_

        def wo_body(n, _, parts=parts, t=t):
            acc = None
            for h in range(H):
                a = jnp.concatenate([qr[h, sl:sl + n_, :] for sl, n_ in parts], axis=0)
                y = _dot(a.astype(BF16), wo[n, h * 64:(h + 1) * 64, :])
                acc = y if acc is None else acc + y
            hbuf[t:t + 128, pl.ds(pl.multiple_of(n * 128, 128), 128)] = acc
        jax.lax.fori_loop(0, ND, wo_body, None, unroll=2)

    for j in range(NF):
        w1_cp(j).wait()
    for n in range(ND):
        w2_cp(n).wait()
    mod_chunk(4)
    mod_chunk(5)
    ga = modv[2][0:1, :]
    sb = modv[3][0:1, :]
    cb = modv[4][0:1, :]
    gb = modv[5][0:1, :]
    b2 = b2_ref[...].astype(F32)

    def out_cp(i):
        r = pl.multiple_of(i * RC, RC)
        return pltpu.make_async_copy(out_ref.at[pl.ds(r, RC)], out_hbm.at[pl.ds(r, RC)], sems.at[4])

    def ffn_body(i, _):
        r = pl.multiple_of(i * RC, RC)
        x1 = x_ref[pl.ds(r, RC), :].astype(F32) + ga * hbuf[pl.ds(r, RC), :]
        h2 = (_ln(x1) * (1.0 + cb) + sb).astype(BF16)
        g = []
        for j in range(NF):
            u = _dot(h2, w1[j]) + b1_ref[:, j * 128:(j + 1) * 128].astype(F32)
            g.append(jax.nn.gelu(u, approximate=True).astype(BF16))
        gg = jnp.concatenate(g, axis=1)
        y = jnp.concatenate([_dot(gg, w2[n]) for n in range(ND)], axis=1)
        out_ref[pl.ds(r, RC), :] = (x1 + gb * (y + b2)).astype(out_ref.dtype)
        out_cp(i).start()
    jax.lax.fori_loop(0, S // RC, ffn_body, None)
    for i in range(S // RC):
        out_cp(i).wait()


@functools.partial(jax.jit, static_argnames=("A_seg_len",))
def pallas_adaLN_cond__memory_aug_recurrent_mem_tr__dense_activation_gelu__prompt_kernel(
    A_x, A_mem0, A_Wq, A_Wk, A_Wv, A_Wo, A_seg_len, B_x, B_w1, B_b1, B_w2, B_b2, c, w_mod,
):
    assert A_seg_len == SEG and A_x.shape == (1, S, D)
    vm = pl.BlockSpec(memory_space=pltpu.VMEM)
    hb = pl.BlockSpec(memory_space=pl.ANY)
    out = pl.pallas_call(
        _kernel,
        out_shape=jax.ShapeDtypeStruct((S, D), A_x.dtype),
        in_specs=[vm] * 5 + [hb] * 7,
        out_specs=hb,
        scratch_shapes=[
            pltpu.VMEM((3 * H, D // 2, E), U32),
            pltpu.VMEM((ND, H * E // 2, 128), U32),
            pltpu.VMEM((NF, D // 2, 128), U32),
            pltpu.VMEM((ND, F // 2, 128), U32),
            pltpu.VMEM((S + 32, D), F32),
            pltpu.VMEM((H, RING, E), F32),
            pltpu.VMEM((H, RING, E), F32),
            pltpu.VMEM((H, RING, E), F32),
            pltpu.VMEM((2, 16, D, 128), U32),
            pltpu.VMEM((2, D, D), BF16),
            pltpu.VMEM((6, 8, D), F32),
            pltpu.VMEM((PRE, D), BF16),
            pltpu.VMEM((S, D), BF16),
            pltpu.SemaphoreType.DMA((18,)),
        ],
        compiler_params=pltpu.CompilerParams(vmem_limit_bytes=126 * 2**20),
    )(A_x.reshape(S, D), A_mem0.reshape(M, D), B_b1.reshape(1, F), B_b2.reshape(1, D), c,
      A_Wq, A_Wk, A_Wv, A_Wo.reshape(H * E, D), B_w1, B_w2, w_mod)
    return out.reshape(1, S, D)
```

```python
import functools

import jax
import jax.numpy as jnp
import jax.experimental.pallas as pl
import jax.experimental.pallas.tpu as pltpu

F32 = jnp.float32
BF16 = jnp.bfloat16
U32 = jnp.uint32

S, D, H, E, M, SEG, F = 2048, 1024, 32, 128, 8, 32, 3584
NSEG = S // SEG
TPS = 24
TAIL = S - NSEG * TPS
PRE = 544
RING = 576
OFF = 32
LAG1, LAG2, LAG3, LAG4 = 4, 8, 12, 16
RC = 256
NF = F // 128
ND = D // 128


def _ln(x):
    m = jnp.mean(x, axis=-1, keepdims=True)
    xc = x - m
    v = jnp.mean(xc * xc, axis=-1, keepdims=True)
    return xc * jax.lax.rsqrt(v + 1e-5)


def _dot(a, b):
    if b.dtype == U32:
        b = pltpu.bitcast(b, BF16)
    return jnp.dot(a, b, preferred_element_type=F32)


def _kernel(mem0_ref, b1_ref, b2_ref, c_ref,
            x_hbm, wq_hbm, wk_hbm, wv_hbm, wo_hbm, w1_hbm, w2_hbm, wm_hbm,
            out_hbm,
            wqkv, wo, w1, w2, hbuf, qr, kr, vr, stg, wm, modv, hb, out_ref, x_ref, sems):
    def wm_cp(j):
        return pltpu.make_async_copy(wm_hbm.at[:, pl.ds(j * D, D)], wm.at[j % 2], sems.at[j % 2])

    def stg_cps(i):
        w32 = (wq_hbm, wk_hbm, wv_hbm)[i].bitcast(U32)
        return [pltpu.make_async_copy(w32.at[:, p, :], stg.at[i % 2, p], sems.at[2 + i % 2])
                for p in range(16)]

    def wo_cp(n):
        return pltpu.make_async_copy(
            wo_hbm.bitcast(U32).at[:, pl.ds(n * 128, 128)], wo.at[n], sems.at[8 + n])

    def w1_cp(j):
        return pltpu.make_async_copy(
            w1_hbm.bitcast(U32).at[:, pl.ds(j * 128, 128)], w1.at[j], sems.at[16])

    def w2_cp(n):
        return pltpu.make_async_copy(
            w2_hbm.bitcast(U32).at[:, pl.ds(n * 128, 128)], w2.at[n], sems.at[17])

    def x_cp(a, b, k):
        return pltpu.make_async_copy(x_hbm.at[a:b], x_ref.at[a:b], sems.at[k])

    wm_cp(0).start()
    wm_cp(1).start()
    x_cp(0, 768, 5).start()
    for i in range(2):
        for cp in stg_cps(i):
            cp.start()

    cc = c_ref[...].astype(F32)
    sc = jnp.broadcast_to(cc * jax.nn.sigmoid(cc), (8, D)).astype(BF16)

    def mod_chunk(j):
        wm_cp(j).wait()
        modv[j] = _dot(sc, wm[j % 2])

    mod_chunk(0)
    mod_chunk(1)
    sa = modv[0][0:1, :]
    ca = modv[1][0:1, :]

    def ln_body(i, _):
        r = pl.multiple_of(i * 256, 256)
        hbuf[pl.ds(r, 256), :] = _ln(x_ref[pl.ds(r, 256), :].astype(F32)) * (1.0 + ca) + sa
    x_cp(0, 768, 5).wait()
    jax.lax.fori_loop(0, 3, ln_body, None)

    hbuf[S:S + 32, :] = jnp.zeros((32, D), F32)

    def relayout16(i, t):
        dd = pl.multiple_of(t * 16, 16)
        d2 = pl.multiple_of(t * 8, 8)
        for p in range(16):
            a = stg[i % 2, p, pl.ds(dd, 8, stride=2), :]
            b = stg[i % 2, p, pl.ds(dd + 1, 8, stride=2), :]
            lo = (a & jnp.uint32(0xFFFF)) | (b << 16)
            hi = (a >> 16) | (b & jnp.uint32(0xFFFF0000))
            wqkv[i * H + 2 * p, pl.ds(d2, 8), :] = lo
            wqkv[i * H + 2 * p + 1, pl.ds(d2, 8), :] = hi

    hb[...] = hbuf[0:PRE, :].astype(BF16)
    rings = (qr, kr, vr)
    for cp in stg_cps(0):
        cp.wait()
    jax.lax.fori_loop(0, 64, lambda t, _: relayout16(0, t), None)
    for cp in stg_cps(2):
        cp.start()
    for i in range(3):
        if i < 2:
            for cp in stg_cps(i + 1):
                cp.wait()
        if i == 1:
            x_cp(768, S, 6).start()
            for n in range(ND):
                wo_cp(n).start()
            wm_cp(2).start()
            wm_cp(3).start()
            for j in range(NF):
                w1_cp(j).start()
            for n in range(ND):
                w2_cp(n).start()

        def pre_body(h, _, i=i):
            lhs = hb[...]
            rings[i][h, OFF:OFF + PRE, :] = _dot(lhs, wqkv[i * H + h])
            if i < 2:
                relayout16(i + 1, 2 * h)
                relayout16(i + 1, 2 * h + 1)
        jax.lax.fori_loop(0, H, pre_body, None, unroll=2)

    x_cp(768, S, 6).wait()
    jax.lax.fori_loop(3, S // 256, ln_body, None)
    for n in range(ND):
        wo_cp(n).wait()

    row = jax.lax.broadcasted_iota(jnp.int32, (M + SEG, M + SEG), 0)
    col = jax.lax.broadcasted_iota(jnp.int32, (M + SEG, M + SEG), 1)
    mask = (row < M) | (row >= col)
    scale = E ** -0.5

    def step(s, mem):
        tin = pl.multiple_of(PRE + s * TPS, 8)
        slot_in = pl.multiple_of(jax.lax.rem(OFF + PRE + s * TPS, RING), 8)
        slot_seg = pl.multiple_of(jax.lax.rem(OFF + s * SEG, RING), 8)
        tout = pl.multiple_of(s * TPS, 8)
        slot_out = pl.multiple_of(jax.lax.rem(OFF + s * TPS, RING), 8)
        slot_out2 = pl.multiple_of(jax.lax.rem(OFF + 16 + s * TPS, RING), 8)
        lhs = jnp.concatenate([mem, hbuf[pl.ds(tin, TPS), :]], axis=0).astype(BF16)
        om = []
        toks = [[rings[i][h, pl.ds(slot_seg, SEG), :] for i in range(3)] for h in range(H)]
        qkv, scs, ps = {}, {}, {}
        outs = [None] * ND

        def st_qkv(h):
            full = []
            for i in range(3):
                y = _dot(lhs, wqkv[i * H + h])
                rings[i][h, pl.ds(slot_in, TPS), :] = y[M:, :]
                full.append(jnp.concatenate([y[:M, :], toks[h][i]], axis=0).astype(BF16))
            qkv[h] = full

        def st_s(h):
            q, k, _ = qkv[h]
            scs[h] = jax.lax.dot_general(q, k, (((1,), (1,)), ((), ())),
                                         preferred_element_type=F32)

        def st_p(h):
            sc_ = jnp.where(mask, scs[h] * scale, -1e9)
            p = jnp.exp(sc_ - jnp.max(sc_, axis=-1, keepdims=True))
            ps[h] = (p / jnp.sum(p, axis=-1, keepdims=True)).astype(BF16)

        def st_o(h):
            o = _dot(ps[h], qkv[h][2])
            qr[h, pl.ds(slot_seg, SEG), :] = o[M:, :]
            om.append(jnp.concatenate(
                [o[:M, :], qr[h, pl.ds(slot_out, 16), :], qr[h, pl.ds(slot_out2, 8), :]],
                axis=0).astype(BF16))

        def st_w(h):
            for n in range(ND):
                y = _dot(om[h], wo[n, h * 64:(h + 1) * 64, :])
                outs[n] = y if outs[n] is None else outs[n] + y

        for t in range(H + LAG4):
            if t < H:
                st_qkv(t)
            if 0 <= t - LAG1 < H:
                st_s(t - LAG1)
            if 0 <= t - LAG2 < H:
                st_p(t - LAG2)
            if 0 <= t - LAG3 < H:
                st_o(t - LAG3)
            if 0 <= t - LAG4 < H:
                st_w(t - LAG4)
        res = jnp.concatenate(outs, axis=1)
        hbuf[pl.ds(tout, TPS), :] = res[M:, :]
        return res[:M, :]

    jax.lax.fori_loop(0, NSEG, step, mem0_ref[...].astype(F32))

    mod_chunk(2)
    mod_chunk(3)
    wm_cp(4).start()
    wm_cp(5).start()
    T0 = NSEG * TPS
    for blk in range(TAIL // 128):
        t = T0 + blk * 128
        parts = []
        left = 128
        while left:
            sl = (OFF + t + 128 - left) % RING
            n_ = min(left, RING - sl)
            parts.append((sl, n_))
            left -= n_

        def wo_body(n, _, parts=parts, t=t):
            acc = None
            for h in range(H):
                a = jnp.concatenate([qr[h, sl:sl + n_, :] for sl, n_ in parts], axis=0)
                y = _dot(a.astype(BF16), wo[n, h * 64:(h + 1) * 64, :])
                acc = y if acc is None else acc + y
            hbuf[t:t + 128, pl.ds(pl.multiple_of(n * 128, 128), 128)] = acc
        jax.lax.fori_loop(0, ND, wo_body, None, unroll=2)

    for j in range(NF):
        w1_cp(j).wait()
    for n in range(ND):
        w2_cp(n).wait()
    mod_chunk(4)
    mod_chunk(5)
    ga = modv[2][0:1, :]
    sb = modv[3][0:1, :]
    cb = modv[4][0:1, :]
    gb = modv[5][0:1, :]
    b2 = b2_ref[...].astype(F32)

    def out_cp(i):
        r = pl.multiple_of(i * RC, RC)
        return pltpu.make_async_copy(out_ref.at[pl.ds(r, RC)], out_hbm.at[pl.ds(r, RC)], sems.at[4])

    def ffn_body(i, _):
        r = pl.multiple_of(i * RC, RC)
        x1 = x_ref[pl.ds(r, RC), :].astype(F32) + ga * hbuf[pl.ds(r, RC), :]
        h2 = (_ln(x1) * (1.0 + cb) + sb).astype(BF16)
        g = []
        for j in range(NF):
            u = _dot(h2, w1[j]) + b1_ref[:, j * 128:(j + 1) * 128].astype(F32)
            g.append(jax.nn.gelu(u, approximate=True).astype(BF16))
        gg = jnp.concatenate(g, axis=1)
        y = jnp.concatenate([_dot(gg, w2[n]) for n in range(ND)], axis=1)
        out_ref[pl.ds(r, RC), :] = (x1 + gb * (y + b2)).astype(out_ref.dtype)
        out_cp(i).start()
    jax.lax.fori_loop(0, S // RC, ffn_body, None)
    for i in range(S // RC):
        out_cp(i).wait()


@functools.partial(jax.jit, static_argnames=("A_seg_len",))
def pallas_adaLN_cond__memory_aug_recurrent_mem_tr__dense_activation_gelu__prompt_kernel(
    A_x, A_mem0, A_Wq, A_Wk, A_Wv, A_Wo, A_seg_len, B_x, B_w1, B_b1, B_w2, B_b2, c, w_mod,
):
    assert A_seg_len == SEG and A_x.shape == (1, S, D)
    vm = pl.BlockSpec(memory_space=pltpu.VMEM)
    hb = pl.BlockSpec(memory_space=pl.ANY)
    out = pl.pallas_call(
        _kernel,
        out_shape=jax.ShapeDtypeStruct((S, D), A_x.dtype),
        in_specs=[vm] * 4 + [hb] * 8,
        out_specs=hb,
        scratch_shapes=[
            pltpu.VMEM((3 * H, D // 2, E), U32),
            pltpu.VMEM((ND, H * E // 2, 128), U32),
            pltpu.VMEM((NF, D // 2, 128), U32),
            pltpu.VMEM((ND, F // 2, 128), U32),
            pltpu.VMEM((S + 32, D), F32),
            pltpu.VMEM((H, RING, E), F32),
            pltpu.VMEM((H, RING, E), F32),
            pltpu.VMEM((H, RING, E), F32),
            pltpu.VMEM((2, 16, D, 128), U32),
            pltpu.VMEM((2, D, D), BF16),
            pltpu.VMEM((6, 8, D), F32),
            pltpu.VMEM((PRE, D), BF16),
            pltpu.VMEM((S, D), BF16),
            pltpu.VMEM((S, D), BF16),
            pltpu.SemaphoreType.DMA((18,)),
        ],
        compiler_params=pltpu.CompilerParams(vmem_limit_bytes=126 * 2**20,
            flags={'XLA_TPU_EVENLY_DISTRIBUTE_CRITICAL_NODES': True}),
    )(A_mem0.reshape(M, D), B_b1.reshape(1, F), B_b2.reshape(1, D), c,
      A_x.reshape(S, D), A_Wq, A_Wk, A_Wv, A_Wo.reshape(H * E, D), B_w1, B_w2, w_mod)
    return out.reshape(1, S, D)
```

```python
import functools

import jax
import jax.numpy as jnp
import jax.experimental.pallas as pl
import jax.experimental.pallas.tpu as pltpu

F32 = jnp.float32
BF16 = jnp.bfloat16
U32 = jnp.uint32

S, D, H, E, M, SEG, F = 2048, 1024, 32, 128, 8, 32, 3584
NSEG = S // SEG
TPS = 24
TAIL = S - NSEG * TPS
PRE = 544
RING = 576
OFF = 32
LAG1, LAG2, LAG3, LAG4 = 4, 8, 12, 16
RC = 128
NF = F // 128
ND = D // 128


def _ln(x):
    m = jnp.mean(x, axis=-1, keepdims=True)
    xc = x - m
    v = jnp.mean(xc * xc, axis=-1, keepdims=True)
    return xc * jax.lax.rsqrt(v + 1e-5)


def _dot(a, b):
    if b.dtype == U32:
        b = pltpu.bitcast(b, BF16)
    return jnp.dot(a, b, preferred_element_type=F32)


def _kernel(mem0_ref, b1_ref, b2_ref, c_ref,
            x_hbm, wq_hbm, wk_hbm, wv_hbm, wo_hbm, w1_hbm, w2_hbm, wm_hbm,
            out_hbm,
            wqkv, wo, w1, w2, hbuf, qr, kr, vr, stg, wm, modv, hb, out_ref, x_ref, sems):
    def wm_cp(j):
        return pltpu.make_async_copy(wm_hbm.at[:, pl.ds(j * D, D)], wm.at[j % 2], sems.at[j % 2])

    def stg_cp(i, p):
        w32 = (wq_hbm, wk_hbm, wv_hbm)[i].bitcast(U32)
        return pltpu.make_async_copy(
            w32.at[:, p, :], stg.at[i % 2, p], sems.at[18 + (i % 2) * 16 + p])

    def wo_cp(n):
        return pltpu.make_async_copy(
            wo_hbm.bitcast(U32).at[:, pl.ds(n * 128, 128)], wo.at[n], sems.at[8 + n])

    def w1_cp(j):
        return pltpu.make_async_copy(
            w1_hbm.bitcast(U32).at[:, pl.ds(j * 128, 128)], w1.at[j], sems.at[16])

    def w2_cp(n):
        return pltpu.make_async_copy(
            w2_hbm.bitcast(U32).at[:, pl.ds(n * 128, 128)], w2.at[n], sems.at[17])

    def x_cp(a, b, k):
        return pltpu.make_async_copy(x_hbm.at[a:b], x_ref.at[a:b], sems.at[k])

    wm_cp(0).start()
    wm_cp(1).start()
    x_cp(0, 768, 5).start()
    for i in range(2):
        for p in range(16):
            stg_cp(i, p).start()

    cc = c_ref[...].astype(F32)
    sc = jnp.broadcast_to(cc * jax.nn.sigmoid(cc), (8, D)).astype(BF16)

    def mod_chunk(j):
        wm_cp(j).wait()
        modv[j] = _dot(sc, wm[j % 2])

    mod_chunk(0)
    mod_chunk(1)
    sa = modv[0][0:1, :]
    ca = modv[1][0:1, :]

    def ln_body(i, _):
        r = pl.multiple_of(i * 256, 256)
        hbuf[pl.ds(r, 256), :] = _ln(x_ref[pl.ds(r, 256), :].astype(F32)) * (1.0 + ca) + sa
    x_cp(0, 768, 5).wait()
    jax.lax.fori_loop(0, 3, ln_body, None)

    hbuf[S:S + 32, :] = jnp.zeros((32, D), F32)

    def relayout(i, p):
        stg_cp(i, p).wait()
        for t in range(D // 16):
            a = stg[i % 2, p, pl.ds(t * 16, 8, stride=2), :]
            b = stg[i % 2, p, pl.ds(t * 16 + 1, 8, stride=2), :]
            wqkv[i * H + 2 * p, t * 8:t * 8 + 8, :] = (a & jnp.uint32(0xFFFF)) | (b << 16)
            wqkv[i * H + 2 * p + 1, t * 8:t * 8 + 8, :] = (a >> 16) | (b & jnp.uint32(0xFFFF0000))
        if i == 0:
            stg_cp(2, p).start()

    hb[...] = hbuf[0:PRE, :].astype(BF16)
    rings = (qr, kr, vr)
    relayout(0, 0)
    for i in range(3):
        if i == 1:
            x_cp(768, S, 6).start()
            for n in range(ND):
                wo_cp(n).start()
        if i == 2:
            wm_cp(2).start()
            wm_cp(3).start()
            for j in range(NF):
                w1_cp(j).start()
            for n in range(ND):
                w2_cp(n).start()

        def pre_pair(p, i=i):
            for u in range(2):
                rings[i][2 * p + u, OFF:OFF + PRE, :] = _dot(hb[...], wqkv[i * H + 2 * p + u])

        def pre_body(p, _, i=i):
            relayout(i, p + 1)
            pre_pair(p)
        jax.lax.fori_loop(0, 15, pre_body, None)
        if i < 2:
            relayout(i + 1, 0)
        pre_pair(15)

    x_cp(768, S, 6).wait()
    jax.lax.fori_loop(3, S // 256, ln_body, None)
    for n in range(ND):
        wo_cp(n).wait()

    row = jax.lax.broadcasted_iota(jnp.int32, (M + SEG, M + SEG), 0)
    col = jax.lax.broadcasted_iota(jnp.int32, (M + SEG, M + SEG), 1)
    mask = (row < M) | (row >= col)
    scale = E ** -0.5

    def step(s, mem):
        tin = pl.multiple_of(PRE + s * TPS, 8)
        slot_in = pl.multiple_of(jax.lax.rem(OFF + PRE + s * TPS, RING), 8)
        slot_seg = pl.multiple_of(jax.lax.rem(OFF + s * SEG, RING), 8)
        tout = pl.multiple_of(s * TPS, 8)
        slot_out = pl.multiple_of(jax.lax.rem(OFF + s * TPS, RING), 8)
        slot_out2 = pl.multiple_of(jax.lax.rem(OFF + 16 + s * TPS, RING), 8)
        lhs = jnp.concatenate([mem, hbuf[pl.ds(tin, TPS), :]], axis=0).astype(BF16)
        om = []
        toks = [[rings[i][h, pl.ds(slot_seg, SEG), :] for i in range(3)] for h in range(H)]
        qkv, scs, ps = {}, {}, {}
        outs = [None] * ND

        def st_qkv(h):
            full = []
            for i in range(3):
                y = _dot(lhs, wqkv[i * H + h])
                rings[i][h, pl.ds(slot_in, TPS), :] = y[M:, :]
                full.append(jnp.concatenate([y[:M, :], toks[h][i]], axis=0))
            qkv[h] = full

        def st_s(h):
            q, k, _ = qkv[h]
            scs[h] = jax.lax.dot_general(q, k, (((1,), (1,)), ((), ())),
                                         preferred_element_type=F32)

        def st_p(h):
            sc_ = jnp.where(mask, scs[h] * scale, -1e9)
            p = jnp.exp(sc_ - jnp.max(sc_, axis=-1, keepdims=True))
            ps[h] = (p / jnp.sum(p, axis=-1, keepdims=True))

        def st_o(h):
            o = _dot(ps[h], qkv[h][2])
            qr[h, pl.ds(slot_seg, SEG), :] = o[M:, :]
            om.append(jnp.concatenate(
                [o[:M, :], qr[h, pl.ds(slot_out, 16), :], qr[h, pl.ds(slot_out2, 8), :]],
                axis=0).astype(BF16))

        def st_w(h):
            for n in range(ND):
                y = _dot(om[h], wo[n, h * 64:(h + 1) * 64, :])
                outs[n] = y if outs[n] is None else outs[n] + y

        for t in range(H + LAG4):
            if t < H:
                st_qkv(t)
            if 0 <= t - LAG1 < H:
                st_s(t - LAG1)
            if 0 <= t - LAG2 < H:
                st_p(t - LAG2)
            if 0 <= t - LAG3 < H:
                st_o(t - LAG3)
            if 0 <= t - LAG4 < H:
                st_w(t - LAG4)
        res = jnp.concatenate(outs, axis=1)
        hbuf[pl.ds(tout, TPS), :] = res[M:, :]
        return res[:M, :]

    jax.lax.fori_loop(0, NSEG, step, mem0_ref[...].astype(F32))

    mod_chunk(2)
    mod_chunk(3)
    wm_cp(4).start()
    wm_cp(5).start()
    T0 = NSEG * TPS
    for blk in range(TAIL // 128):
        t = T0 + blk * 128
        parts = []
        left = 128
        while left:
            sl = (OFF + t + 128 - left) % RING
            n_ = min(left, RING - sl)
            parts.append((sl, n_))
            left -= n_

        def wo_body(n, _, parts=parts, t=t):
            acc = None
            for h in range(H):
                a = jnp.concatenate([qr[h, sl:sl + n_, :] for sl, n_ in parts], axis=0)
                y = _dot(a.astype(BF16), wo[n, h * 64:(h + 1) * 64, :])
                acc = y if acc is None else acc + y
            hbuf[t:t + 128, pl.ds(pl.multiple_of(n * 128, 128), 128)] = acc
        jax.lax.fori_loop(0, ND, wo_body, None, unroll=2)

    for j in range(NF):
        w1_cp(j).wait()
    for n in range(ND):
        w2_cp(n).wait()
    mod_chunk(4)
    mod_chunk(5)
    ga = modv[2][0:1, :]
    sb = modv[3][0:1, :]
    cb = modv[4][0:1, :]
    gb = modv[5][0:1, :]
    b2 = b2_ref[...].astype(F32)

    def out_cp(i):
        r = pl.multiple_of(i * RC, RC)
        return pltpu.make_async_copy(out_ref.at[pl.ds(r, RC)], out_hbm.at[pl.ds(r, RC)], sems.at[4])

    def ffn_body(i, _):
        r = pl.multiple_of(i * RC, RC)
        x1 = x_ref[pl.ds(r, RC), :].astype(F32) + ga * hbuf[pl.ds(r, RC), :]
        h2 = (_ln(x1) * (1.0 + cb) + sb).astype(BF16)
        g = []
        for j in range(NF):
            u = _dot(h2, w1[j]) + b1_ref[:, j * 128:(j + 1) * 128].astype(F32)
            g.append(jax.nn.gelu(u, approximate=True).astype(BF16))
        gg = jnp.concatenate(g, axis=1)
        y = jnp.concatenate([_dot(gg, w2[n]) for n in range(ND)], axis=1)
        out_ref[pl.ds(r, RC), :] = (x1 + gb * (y + b2)).astype(out_ref.dtype)
        out_cp(i).start()
    jax.lax.fori_loop(0, S // RC, ffn_body, None, unroll=2)
    for i in range(S // RC):
        out_cp(i).wait()


@functools.partial(jax.jit, static_argnames=("A_seg_len",))
def pallas_adaLN_cond__memory_aug_recurrent_mem_tr__dense_activation_gelu__prompt_kernel(
    A_x, A_mem0, A_Wq, A_Wk, A_Wv, A_Wo, A_seg_len, B_x, B_w1, B_b1, B_w2, B_b2, c, w_mod,
):
    assert A_seg_len == SEG and A_x.shape == (1, S, D)
    vm = pl.BlockSpec(memory_space=pltpu.VMEM)
    hb = pl.BlockSpec(memory_space=pl.ANY)
    out = pl.pallas_call(
        _kernel,
        out_shape=jax.ShapeDtypeStruct((S, D), A_x.dtype),
        in_specs=[vm] * 4 + [hb] * 8,
        out_specs=hb,
        scratch_shapes=[
            pltpu.VMEM((3 * H, D // 2, E), U32),
            pltpu.VMEM((ND, H * E // 2, 128), U32),
            pltpu.VMEM((NF, D // 2, 128), U32),
            pltpu.VMEM((ND, F // 2, 128), U32),
            pltpu.VMEM((S + 32, D), F32),
            pltpu.VMEM((H, RING, E), F32),
            pltpu.VMEM((H, RING, E), F32),
            pltpu.VMEM((H, RING, E), F32),
            pltpu.VMEM((2, 16, D, 128), U32),
            pltpu.VMEM((2, D, D), BF16),
            pltpu.VMEM((6, 8, D), F32),
            pltpu.VMEM((PRE, D), BF16),
            pltpu.VMEM((S, D), BF16),
            pltpu.VMEM((S, D), BF16),
            pltpu.SemaphoreType.DMA((50,)),
        ],
        compiler_params=pltpu.CompilerParams(vmem_limit_bytes=126 * 2**20,
            flags={'XLA_TPU_EVENLY_DISTRIBUTE_CRITICAL_NODES': True}),
    )(A_mem0.reshape(M, D), B_b1.reshape(1, F), B_b2.reshape(1, D), c,
      A_x.reshape(S, D), A_Wq, A_Wk, A_Wv, A_Wo.reshape(H * E, D), B_w1, B_w2, w_mod)
    return out.reshape(1, S, D)
```
